```python
import jax
import jax.numpy as jnp

def _softmax(x, axis=-1):
    return jax.nn.softmax(x, axis=axis)
def _gelu(x):
    return jax.nn.gelu(x, approximate=True)
def _silu(x):
    return jax.nn.silu(x)
def _sigmoid(x):
    return jax.nn.sigmoid(x)
def _layernorm(x, axis=-1, eps=1e-5):
    m = jnp.mean(x, axis=axis, keepdims=True)
    v = jnp.var(x, axis=axis, keepdims=True)
    return (x - m) / jnp.sqrt(v + eps)
def _scatter_add(tgt, idx, src, axis=0):
    return tgt.at[idx].add(src)
def _segment_sum(src, seg, n):
    return jax.ops.segment_sum(src, seg, n)
class _Rng:
    def __init__(self, key):
        self._k = key
    def _next(self):
        self._k, sub = jax.random.split(self._k)
        return sub
    def normal(self, shape):
        return jax.random.normal(self._next(), shape, dtype=jnp.bfloat16)
    def randint(self, lo, hi, shape):
        return jax.random.randint(self._next(), shape, lo, hi, dtype=jnp.int32)
    def uniform(self, shape, lo=0.0, hi=1.0):
        return jax.random.uniform(self._next(), shape, jnp.bfloat16, lo, hi)
    def permutation(self, n):
        return jax.random.permutation(self._next(), n)


kernel_name = 'recurrent_scan__sliding_block_cached__moe_arch_mod__decode'

def setup_inputs():
    _rng = _Rng(jax.random.key(int.from_bytes(__import__("os").urandom(4), "little")))
    _w = (lambda a: (lambda t: t.astype(jnp.bfloat16) if jnp.issubdtype(t.dtype, jnp.floating) else t)(jnp.asarray(a)))
    def _A_setup():
        B, Sq, D = 1, 1, 512
        Hq, Hkv, Sk, Dh = 32, 32, 32768, 128
        assert Hq % Hkv == 0, (Hq, Hkv)
        return {
            "x": _w((lambda *s: _rng.normal(s) * 0.05)(B, Sq, D)),
            "k_cache": _w((lambda *s: _rng.normal(s) * 0.05)(B, Hkv, Sk, Dh)),
            "v_cache": _w((lambda *s: _rng.normal(s) * 0.05)(B, Hkv, Sk, Dh)),
            "wq": _w((lambda *s: _rng.normal(s) * 0.05)(D, Hq * Dh) * (D ** -0.5)),
            "wo": _w((lambda *s: _rng.normal(s) * 0.05)(Hq * Dh, D) * ((Hq * Dh) ** -0.5)),
        }
    _A_in = _A_setup()

    def _B_setup():
        B, S, D, F, C = 1, 1, 512, 1376, 1
        return {
            "x": _w((lambda *s: _rng.normal(s) * 0.05)(B, S, D)),
            "w_r": _w((lambda *s: _rng.normal(s) * 0.05)(D)),
            "w_gate": _w((lambda *s: _rng.normal(s) * 0.05)(D, F)),
            "w_up": _w((lambda *s: _rng.normal(s) * 0.05)(D, F)),
            "w_down": _w((lambda *s: _rng.normal(s) * 0.05)(F, D)),
        }
    _B_in = _B_setup()

    return {
        "A_x": _A_in["x"],
        "A_k_cache": _A_in["k_cache"],
        "A_v_cache": _A_in["v_cache"],
        "A_wq": _A_in["wq"],
        "A_wo": _A_in["wo"],
        "B_x": _B_in["x"],
        "B_w_r": _B_in["w_r"],
        "B_w_gate": _B_in["w_gate"],
        "B_w_up": _B_in["w_up"],
        "B_w_down": _B_in["w_down"],
    }

def reference(A_x, A_k_cache, A_v_cache, A_wq, A_wo, B_x, B_w_r, B_w_gate, B_w_up, B_w_down):
    def _A_ref(x, k_cache, v_cache, wq, wo):
        B, Sq, D = x.shape
        Hq, Dh = 32, 128
        Hkv, Sk = k_cache.shape[1], k_cache.shape[2]
        W = min(4096, max(256, Sk // 4))
        rep = Hq // Hkv
        q = (lambda x, *d: x.transpose(*d))((x @ wq).reshape(B, Sq, Hq, Dh), 0, 2, 1, 3)
        k = jnp.repeat(k_cache[:, :, Sk - W:, :], rep, axis=1)
        v = jnp.repeat(v_cache[:, :, Sk - W:, :], rep, axis=1)
        scores = jnp.einsum("bhqd,bhkd->bhqk", q, k) * (Dh ** -0.5)
        p = _softmax(scores, axis=-1)
        o = jnp.einsum("bhqk,bhkd->bhqd", p, v)
        return (lambda x, *d: x.transpose(*d))(o, 0, 2, 1, 3).reshape(B, Sq, Hq * Dh) @ wo

    def _B_ref(x, w_r, w_gate, w_up, w_down):
        B, S, D = x.shape
        C = 1
        r = x @ w_r
        idx = jnp.argsort(-r, axis=-1)[:, :C]
        idx_e = jnp.repeat(idx.reshape(B, C, 1), D, axis=2)
        x_sel = jnp.take_along_axis(x, idx_e, axis=1)
        g = _silu(x_sel @ w_gate)
        u = x_sel @ w_up
        y = (g * u) @ w_down
        r_sel = _sigmoid(jnp.take_along_axis(r, idx, axis=1))
        y = y * r_sel.reshape(B, C, 1)
        b_off = (jnp.arange(B) * S).reshape(B, 1)
        flat_idx = (idx + b_off).reshape(B * C)
        zero = (x * 0.0).reshape(B * S, D)
        upd = _scatter_add(zero, flat_idx, y.reshape(B * C, D), axis=0)
        return x + upd.reshape(B, S, D)

    x = A_x
    xn = _layernorm(x, axis=-1)
    s = _A_ref(xn, A_k_cache, A_v_cache, A_wq, A_wo)
    g = _silu(_B_ref(xn, B_w_r, B_w_gate, B_w_up, B_w_down))
    return x + s * g
```

```python
import functools

import jax
import jax.numpy as jnp
from jax import lax
import jax.experimental.pallas as pl
import jax.experimental.pallas.tpu as pltpu

_F32 = jnp.float32
_BF16 = jnp.bfloat16
_NT = (((1,), (1,)), ((), ()))


def _make_kernel(D, H, SK, DH, W, F, NBUF, WO_CHUNKS, FFN_AT):
    scale = DH ** -0.5
    wo_rows = (H * DH) // WO_CHUNKS

    def kernel(x_hbm, k_hbm, v_hbm, wq_hbm, wo_hbm, wr_hbm, wg_hbm, wu_hbm, wd_hbm,
               o_ref,
               x_v, wr_v, wq_v, wo_v, wg_v, wu_v, wd_v, kbuf, vbuf, q_s, o_s, g_s,
               sem_misc, sem_k, sem_v, sem_wo):
        def k_copy(h, slot):
            return pltpu.make_async_copy(
                k_hbm.at[0, h, pl.ds(SK - W, W), :], kbuf.at[slot], sem_k.at[slot])

        def v_copy(h, slot):
            return pltpu.make_async_copy(
                v_hbm.at[0, h, pl.ds(SK - W, W), :], vbuf.at[slot], sem_v.at[slot])

        def wo_copy(c):
            return pltpu.make_async_copy(
                wo_hbm.at[pl.ds(c * wo_rows, wo_rows), :],
                wo_v.at[pl.ds(c * wo_rows, wo_rows), :], sem_wo.at[c])

        x_cp = pltpu.make_async_copy(x_hbm, x_v, sem_misc.at[0])
        wr_cp = pltpu.make_async_copy(wr_hbm, wr_v, sem_misc.at[1])
        wq_cp = pltpu.make_async_copy(wq_hbm, wq_v, sem_misc.at[2])
        wg_cp = pltpu.make_async_copy(wg_hbm, wg_v, sem_misc.at[3])
        wu_cp = pltpu.make_async_copy(wu_hbm, wu_v, sem_misc.at[4])
        wd_cp = pltpu.make_async_copy(wd_hbm, wd_v, sem_misc.at[5])

        wq_cp.start()
        x_cp.start()
        wr_cp.start()
        wg_cp.start()
        wu_cp.start()
        wd_cp.start()
        for h in range(NBUF):
            k_copy(h, h).start()
            v_copy(h, h).start()

        x_cp.wait()
        x = x_v[0].astype(_F32)
        mu = jnp.mean(x, axis=-1, keepdims=True)
        xc = x - mu
        var = jnp.mean(xc * xc, axis=-1, keepdims=True)
        xn = xc / jnp.sqrt(var + 1e-5)
        xn_b = xn.astype(_BF16)
        xn8 = jnp.broadcast_to(xn_b, (8, D))

        wq_cp.wait()
        q = jnp.dot(xn8, wq_v[...], preferred_element_type=_F32)
        for h in range(H):
            q_s[h] = q[:, h * DH:(h + 1) * DH]

        wr_cp.wait()
        xnf = xn_b.astype(_F32)
        r = jnp.sum(xnf * wr_v[...].astype(_F32).reshape(1, D), axis=-1, keepdims=True)
        wg_cp.wait()
        gt = lax.dot_general(xn8, wg_v[...], _NT, preferred_element_type=_F32)
        wu_cp.wait()
        up = lax.dot_general(xn8, wu_v[...], _NT, preferred_element_type=_F32)
        hh = (gt * jax.nn.sigmoid(gt) * up).astype(_BF16)
        wd_cp.wait()
        y = jnp.dot(hh, wd_v[...], preferred_element_type=_F32)
        z = xnf + y * jax.nn.sigmoid(r)
        g_s[...] = z * jax.nn.sigmoid(z)

        def body(h, carry):
            slot = h % NBUF
            k_copy(h, slot).wait()
            qh = q_s[h].astype(_BF16)
            s = lax.dot_general(qh, kbuf[slot], (((1,), (1,)), ((), ())),
                                preferred_element_type=_F32)

            @pl.when(h + NBUF < H)
            def _():
                k_copy(h + NBUF, slot).start()

            m = jnp.max(s, axis=-1, keepdims=True)
            p = jnp.exp((s - m) * scale)
            l = jnp.sum(p, axis=-1, keepdims=True)
            v_copy(h, slot).wait()
            o = jnp.dot(p.astype(_BF16), vbuf[slot], preferred_element_type=_F32)

            @pl.when(h + NBUF < H)
            def _():
                v_copy(h + NBUF, slot).start()

            @pl.when(h + NBUF == H)
            def _():
                for c in range(WO_CHUNKS):
                    wo_copy(c).start()

            o_s[h] = o / l
            return carry

        lax.fori_loop(0, H, body, 0)

        acc = jnp.zeros((8, D), _F32)
        hpc = H // WO_CHUNKS
        for c in range(WO_CHUNKS):
            oc = jnp.concatenate([o_s[c * hpc + j] for j in range(hpc)], axis=-1).astype(_BF16)
            wo_copy(c).wait()
            acc = acc + jnp.dot(oc, wo_v[pl.ds(c * wo_rows, wo_rows), :],
                                preferred_element_type=_F32)
        res = x + acc[0:1, :] * g_s[0:1, :]
        o_ref[0] = res.astype(o_ref.dtype)

    return kernel


@jax.jit
def pallas_recurrent_scan__sliding_block_cached__moe_arch_mod__decode_kernel(
    A_x: jax.Array,
    A_k_cache: jax.Array,
    A_v_cache: jax.Array,
    A_wq: jax.Array,
    A_wo: jax.Array,
    B_x: jax.Array,
    B_w_r: jax.Array,
    B_w_gate: jax.Array,
    B_w_up: jax.Array,
    B_w_down: jax.Array,
):
    _, _, D = A_x.shape
    _, H, SK, DH = A_k_cache.shape
    W = min(4096, max(256, SK // 4))
    F = B_w_gate.shape[1]
    NBUF = 4
    WO_CHUNKS = 8
    kernel = _make_kernel(D, H, SK, DH, W, F, NBUF, WO_CHUNKS, 0)
    any_spec = pl.BlockSpec(memory_space=pltpu.MemorySpace.HBM)
    return pl.pallas_call(
        kernel,
        out_shape=jax.ShapeDtypeStruct(A_x.shape, A_x.dtype),
        in_specs=[any_spec] * 9,
        out_specs=pl.BlockSpec(memory_space=pltpu.VMEM),
        scratch_shapes=[
            pltpu.VMEM((1, 1, D), _BF16),
            pltpu.VMEM((D,), _BF16),
            pltpu.VMEM((D, H * DH), _BF16),
            pltpu.VMEM((H * DH, D), _BF16),
            pltpu.VMEM((F, D), _BF16),
            pltpu.VMEM((F, D), _BF16),
            pltpu.VMEM((F, D), _BF16),
            pltpu.VMEM((NBUF, W, DH), _BF16),
            pltpu.VMEM((NBUF, W, DH), _BF16),
            pltpu.VMEM((H, 8, DH), _F32),
            pltpu.VMEM((H, 8, DH), _F32),
            pltpu.VMEM((8, D), _F32),
            pltpu.SemaphoreType.DMA((6,)),
            pltpu.SemaphoreType.DMA((NBUF,)),
            pltpu.SemaphoreType.DMA((NBUF,)),
            pltpu.SemaphoreType.DMA((WO_CHUNKS,)),
        ],
        compiler_params=pltpu.CompilerParams(vmem_limit_bytes=64 * 1024 * 1024),
    )(A_x, A_k_cache, A_v_cache, A_wq, A_wo, B_w_r, B_w_gate.T, B_w_up.T, B_w_down)
```

```python
import functools

import jax
import jax.numpy as jnp
from jax import lax
import jax.experimental.pallas as pl
import jax.experimental.pallas.tpu as pltpu

_F32 = jnp.float32
_BF16 = jnp.bfloat16
_NT = (((1,), (1,)), ((), ()))

_HI = 0
_LO = 1


def _make_kernel(D, H, SK, DH, W, F, DEPTH):
    scale = DH ** -0.5
    G = 8
    NG = H // G
    RS = 64
    SH = 16
    NS = W // RS
    NT = NS // 2
    GC = G * DH
    FT = (F + 127) // 128
    FP = FT * 128
    F24 = (F - NS * 16) // 8
    assert F24 * 24 + (NS - F24) * 16 == F and 0 <= F24 <= NS
    QS = D // RS
    WO_Q0 = QS * 16
    WO_K = NS * 24
    WO_V = NS * 24
    WO_TAIL0 = WO_Q0 + WO_K + WO_V
    OS = (H * DH - WO_TAIL0) // DH
    assert WO_TAIL0 % DH == 0 and OS >= 1

    phases = [("Q", 0, QS)]
    for g in range(NG):
        phases += [("K", g, NS), ("V", g, NS)]
    phases += [("O", NG - 1, OS)]
    base = [0]
    for p in phases:
        base.append(base[-1] + p[2])

    def kernel(x_hbm, k_hbm, v_hbm, wq_hbm, wo_hbm, wr_hbm, wg_hbm, wu_hbm, wd_hbm,
               o_ref,
               x_v, wr_v, wq_v, wo_v, wg_v, wu_v, wd_v, kbuf, vbuf,
               xn_s, q_s, s_s, m_s, o_s, h_s, y_s, a_s,
               sem_l, sem_h, sem_x):
        row = lax.broadcasted_iota(jnp.int32, (G, DH), 0)

        def mult(x, m):
            return x if isinstance(x, int) else pl.multiple_of(x, m)

        def l_dst(p, s):
            kind = phases[p][0]
            if kind == "Q":
                return wq_v.at[0, pl.ds(mult(s * RS, RS), RS), :]
            if kind == "O":
                return wo_v.at[pl.ds(mult(WO_TAIL0 + s * DH, DH), DH), :]
            dst = kbuf if kind == "K" else vbuf
            return dst.at[:, pl.ds(mult(s * RS, RS), RS), :]

        def l_wait(p, s):
            dst = l_dst(p, s)
            pltpu.make_async_copy(dst, dst, sem_l.at[(base[p] + s) % DEPTH]).wait()

        def l_start(p, s, c=True):
            kind, g, _ = phases[p]
            sem = sem_l.at[(base[p] + s) % DEPTH]
            if kind == "Q":
                src = wq_hbm.at[pl.ds(mult(s * RS, RS), RS), pl.ds(0, GC)]
                cond(c, lambda: pltpu.make_async_copy(src, l_dst(p, s), sem).start(priority=_LO))
                return
            if kind == "O":
                src = wo_hbm.at[pl.ds(mult(WO_TAIL0 + s * DH, DH), DH), :]
                cond(c, lambda: pltpu.make_async_copy(src, l_dst(p, s), sem).start(priority=_LO))
                return
            src, dst = (k_hbm, kbuf) if kind == "K" else (v_hbm, vbuf)

            def piece(r_src, r_dst, n):
                pltpu.make_async_copy(
                    src.at[0, pl.ds(g * G, G), pl.ds(SK - W + r_src, n), :],
                    dst.at[:, pl.ds(r_dst, n), :], sem).start(priority=_LO)

            def body():
                piece(mult(s * RS + SH, 8), mult(s * RS, RS), RS)

            def last():
                piece(W - RS + SH, W - RS, RS - SH)
                piece(0, W - SH, SH)

            if SH == 0:
                cond(c, body)
            else:
                cond(land(c, s < NS - 1), body)
                cond(land(c, s == NS - 1), last)

        def land(a, b):
            if isinstance(a, bool):
                return b if a else False
            if isinstance(b, bool):
                return a if b else False
            return jnp.logical_and(a, b)

        def cond(c, f):
            if isinstance(c, bool):
                if c:
                    f()
            else:
                pl.when(c)(f)

        def l_issue_ahead(p, s):
            n = phases[p][2]
            t = s + DEPTH
            if n > DEPTH:
                l_start(p, t, t < n)
            if p + 1 < len(phases):
                n1 = phases[p + 1][2]
                c = t >= n
                if n1 < DEPTH:
                    c = land(c, t - n < n1)
                l_start(p + 1, t - n, c)

        def rows_copy(src, dst, r, n, sem):
            return pltpu.make_async_copy(src.at[pl.ds(r, n), :], dst.at[pl.ds(r, n), :], sem)

        ffn = [(wg_hbm, wg_v), (wu_hbm, wu_v), (wd_hbm, wd_v)]

        def h_issue(p, s):
            kind, g, _ = phases[p]
            sem = sem_h.at[p]
            if kind == "Q":
                rows_copy(wo_hbm, wo_v, mult(s * 16, 16), 16, sem).start(priority=_HI)
            elif kind == "K" and g + 1 < NG:
                r = mult(s * 8, 8)
                pltpu.make_async_copy(
                    wq_hbm.at[pl.ds(r, 8), pl.ds((g + 1) * GC, GC)],
                    wq_v.at[g + 1, pl.ds(r, 8), :], sem).start(priority=_HI)
            elif kind == "K":
                rows_copy(wo_hbm, wo_v, mult(WO_Q0 + s * 24, 8), 24, sem).start(priority=_HI)
            elif kind == "V" and g + 1 < NG:
                src, dst = ffn[g]
                cond(s < F24, lambda: rows_copy(src, dst, mult(s * 24, 8), 24, sem).start(priority=_HI))
                cond(s >= F24, lambda: rows_copy(
                    src, dst, mult(F24 * 24 + (s - F24) * 16, 8), 16, sem).start(priority=_HI))
            elif kind == "V":
                half = NS // 2
                r = mult(WO_Q0 + WO_K + s * 24, 8)
                cond(s < half, lambda: rows_copy(wo_hbm, wo_v, r, 24, sem).start(priority=_HI))
                cond(s >= half, lambda: rows_copy(wo_hbm, wo_v, r, 24, sem_h.at[p + 1]).start(priority=_HI))

        def h_wait(p, ref):
            pltpu.make_async_copy(ref, ref, sem_h.at[p]).wait()

        def step(p, s):
            l_wait(p, s)
            h_issue(p, s)
            l_issue_ahead(p, s)

        def pick_rows(r):
            out = r[:, 0:DH]
            for i in range(1, G):
                out = jnp.where(row == i, r[:, i * DH:(i + 1) * DH], out)
            return out

        def qproj(g, k):
            r0 = mult(k * 128, 128)
            r = jnp.dot(xn_s[k].astype(_BF16), wq_v[g, pl.ds(r0, 128), :],
                        preferred_element_type=_F32)
            return pick_rows(r)

        def xn_full():
            return jnp.concatenate([xn_s[k] for k in range(D // 128)], axis=1)

        def woproj(h):
            r0 = mult(h * DH, DH)
            oh = jnp.broadcast_to(o_s[pl.ds(h, 1), :], (8, DH)).astype(_BF16)
            return jnp.dot(oh, wo_v[pl.ds(r0, DH), :], preferred_element_type=_F32)

        x_cp = pltpu.make_async_copy(x_hbm, x_v, sem_x.at[0])
        wr_cp = pltpu.make_async_copy(wr_hbm, wr_v, sem_x.at[1])
        x_cp.start(priority=_HI)
        for s in range(DEPTH):
            if s < QS:
                l_start(0, s)
            else:
                l_start(1, s - QS)
        wr_cp.start(priority=_HI)
        if FP > F:
            for _, dst in ffn:
                dst[pl.ds(F, FP - F), :] = jnp.zeros((FP - F, D), _BF16)

        x_cp.wait()
        x = x_v[0].astype(_F32)
        mu = jnp.mean(x, axis=-1, keepdims=True)
        xc = x - mu
        var = jnp.mean(xc * xc, axis=-1, keepdims=True)
        xn = (xc / jnp.sqrt(var + 1e-5)).astype(_BF16).astype(_F32)
        xn8 = jnp.broadcast_to(xn, (8, D))
        for k in range(D // 128):
            xn_s[k] = xn8[:, k * 128:(k + 1) * 128]

        q = None
        for t in range(QS // 2):
            step(0, 2 * t)
            step(0, 2 * t + 1)
            part = qproj(0, t)
            q = part if q is None else q + part
        q_s[...] = q

        carry_acc = None
        for g in range(NG):
            pk, pv = 1 + 2 * g, 2 + 2 * g

            def k_extra(t, g=g, pk=pk):
                if g == 0:
                    return
                idx = t - 1
                src = ffn[g - 1][1]

                @pl.when(t == 1)
                def _():
                    h_wait(pk - 1, src.at[pl.ds(0, F), :])

                @pl.when(jnp.logical_and(t >= 1, t <= FT))
                def _():
                    r0 = pl.multiple_of(idx * 128, 128)
                    w = src[pl.ds(r0, 128), :]
                    if g == 1:
                        h_s[idx] = lax.dot_general(xn_full().astype(_BF16), w, _NT,
                                                   preferred_element_type=_F32)
                    elif g == 2:
                        up = lax.dot_general(xn_full().astype(_BF16), w, _NT,
                                             preferred_element_type=_F32)
                        gt = h_s[idx]
                        h_s[idx] = gt * jax.nn.sigmoid(gt) * up
                    else:
                        y_s[...] += jnp.dot(h_s[idx].astype(_BF16), w, preferred_element_type=_F32)

                if g == NG - 1:
                    @pl.when(t == 0)
                    def _():
                        y_s[...] = jnp.zeros((8, D), _F32)

                    @pl.when(t == FT + 1)
                    def _():
                        wr_cp.wait()
                        xf = xn_full()
                        r = jnp.sum(xf * wr_v[...].astype(_F32).reshape(1, D), axis=-1, keepdims=True)
                        z = xf + y_s[...] * jax.nn.sigmoid(r)
                        y_s[...] = z * jax.nn.sigmoid(z)

            qb = q_s[...].astype(_BF16)

            def k_body(t, m, g=g, pk=pk, qb=qb, k_extra=k_extra):
                step(pk, 2 * t)
                k_extra(t)
                step(pk, 2 * t + 1)
                r0 = pl.multiple_of(t * 128, 128)
                kt = kbuf[:, pl.ds(r0, 128), :].reshape(G * 128, DH)
                s = pick_rows(lax.dot_general(qb, kt, _NT, preferred_element_type=_F32))
                s_s[t] = s
                return jnp.maximum(m, s)

            m = lax.fori_loop(0, NT, k_body, jnp.full((G, DH), -jnp.inf, _F32))
            m_s[...] = m

            def v_extra(t, g=g, pv=pv):
                @pl.when(t == 0)
                def _():
                    m_s[...] = jnp.broadcast_to(
                        jnp.max(m_s[...], axis=-1, keepdims=True), (G, DH))

                if g + 1 < NG:
                    @pl.when(t == 1)
                    def _():
                        h_wait(pv - 1, wq_v.at[g + 1])
                        q_s[...] = jnp.zeros((G, DH), _F32)

                    @pl.when(jnp.logical_and(t >= 1, t <= D // 128))
                    def _():
                        q_s[...] += qproj(g + 1, t - 1)
                else:
                    n1 = (WO_Q0 + WO_K) // DH
                    n2 = (WO_Q0 + WO_K + WO_V // 2) // DH
                    t2 = NT // 2 + 1

                    @pl.when(t == 1)
                    def _():
                        h_wait(0, wo_v.at[pl.ds(0, WO_Q0), :])
                        h_wait(pv - 1, wo_v.at[pl.ds(WO_Q0, WO_K), :])
                        a_s[...] = jnp.zeros((8, D), _F32)

                    @pl.when(t == t2)
                    def _():
                        h_wait(pv, wo_v.at[pl.ds(WO_Q0 + WO_K, WO_V // 2), :])

                    assert n1 + 1 <= t2
                    @pl.when(jnp.logical_or(jnp.logical_and(t >= 1, t <= n1),
                                            jnp.logical_and(t >= t2, t < t2 + n2 - n1)))
                    def _():
                        h = jnp.where(t <= n1, t - 1, t - t2 + n1)
                        a_s[...] += woproj(h)

            def v_body(t, carry, g=g, pv=pv, v_extra=v_extra):
                acc, l = carry
                step(pv, 2 * t)
                v_extra(t)
                step(pv, 2 * t + 1)
                r0 = pl.multiple_of(t * 128, 128)
                p = jnp.exp((s_s[t] - m_s[...]) * scale)
                vt = jnp.concatenate([vbuf[i, pl.ds(r0, 128), :] for i in range(G)], axis=1)
                r = jnp.dot(p.astype(_BF16), vt, preferred_element_type=_F32)
                return acc + pick_rows(r), l + p

            zero = jnp.zeros((G, DH), _F32)
            acc, l = lax.fori_loop(0, NT, v_body, (zero, zero))
            o_s[pl.ds(g * G, G), :] = acc / jnp.sum(l, axis=-1, keepdims=True)

        po = len(phases) - 1
        n2 = (WO_Q0 + WO_K + WO_V // 2) // DH
        n3 = WO_TAIL0 // DH
        h_wait(po, wo_v.at[pl.ds(WO_Q0 + WO_K + WO_V // 2, WO_V // 2), :])
        a = a_s[...]
        for h in range(n2, n3):
            a = a + woproj(h)
        for s in range(OS):
            l_wait(po, s)
            a = a + woproj(n3 + s)
        res = x_v[0].astype(_F32) + a[0:1, :] * y_s[0:1, :]
        o_ref[0] = res.astype(o_ref.dtype)

    scratch = [
        pltpu.VMEM((1, 1, D), _BF16),
        pltpu.VMEM((D,), _BF16),
        pltpu.VMEM((NG, D, GC), _BF16),
        pltpu.VMEM((H * DH, D), _BF16),
        pltpu.VMEM((FP, D), _BF16),
        pltpu.VMEM((FP, D), _BF16),
        pltpu.VMEM((FP, D), _BF16),
        pltpu.VMEM((G, W, DH), _BF16),
        pltpu.VMEM((G, W, DH), _BF16),
        pltpu.VMEM((D // 128, 8, 128), _F32),
        pltpu.VMEM((G, DH), _F32),
        pltpu.VMEM((NT, G, 128), _F32),
        pltpu.VMEM((G, DH), _F32),
        pltpu.VMEM((H, DH), _F32),
        pltpu.VMEM((FT, 8, 128), _F32),
        pltpu.VMEM((8, D), _F32),
        pltpu.VMEM((8, D), _F32),
        pltpu.SemaphoreType.DMA((DEPTH,)),
        pltpu.SemaphoreType.DMA((len(phases),)),
        pltpu.SemaphoreType.DMA((2,)),
    ]
    return kernel, scratch


@jax.jit
def pallas_recurrent_scan__sliding_block_cached__moe_arch_mod__decode_kernel(
    A_x: jax.Array,
    A_k_cache: jax.Array,
    A_v_cache: jax.Array,
    A_wq: jax.Array,
    A_wo: jax.Array,
    B_x: jax.Array,
    B_w_r: jax.Array,
    B_w_gate: jax.Array,
    B_w_up: jax.Array,
    B_w_down: jax.Array,
):
    _, _, D = A_x.shape
    _, H, SK, DH = A_k_cache.shape
    W = min(4096, max(256, SK // 4))
    F = B_w_gate.shape[1]
    kernel, scratch = _make_kernel(D, H, SK, DH, W, F, DEPTH=8)
    hbm = pl.BlockSpec(memory_space=pltpu.MemorySpace.HBM)
    return pl.pallas_call(
        kernel,
        out_shape=jax.ShapeDtypeStruct(A_x.shape, A_x.dtype),
        in_specs=[hbm] * 9,
        out_specs=pl.BlockSpec(memory_space=pltpu.VMEM),
        scratch_shapes=scratch,
        compiler_params=pltpu.CompilerParams(
            vmem_limit_bytes=64 * 1024 * 1024,
            disable_bounds_checks=True,
        ),
    )(A_x, A_k_cache, A_v_cache, A_wq, A_wo, B_w_r, B_w_gate.T, B_w_up.T, B_w_down)
```

```python
import functools

import jax
import jax.numpy as jnp
from jax import lax
import jax.experimental.pallas as pl
import jax.experimental.pallas.tpu as pltpu

_F32 = jnp.float32
_BF16 = jnp.bfloat16
_NT = (((1,), (1,)), ((), ()))

_HI = 0
_LO = 1


def _make_kernel(D, H, SK, DH, W, F, DEPTH):
    scale = DH ** -0.5
    G = 8
    NG = H // G
    RS = 64
    SH = 16
    NS = W // RS
    NT = NS // 2
    GC = G * DH
    FT = (F + 127) // 128
    FP = FT * 128
    F24 = (F - NS * 16) // 8
    assert F24 * 24 + (NS - F24) * 16 == F and 0 <= F24 <= NS
    QS = D // RS
    WO_Q0 = QS * 16
    WO_K = NS * 24
    WO_V = NS * 24
    WO_TAIL0 = WO_Q0 + WO_K + WO_V
    OS = (H * DH - WO_TAIL0) // DH
    assert WO_TAIL0 % DH == 0 and OS >= 1

    phases = [("Q", 0, QS)]
    for g in range(NG):
        phases += [("K", g, NS), ("V", g, NS)]
    phases += [("O", NG - 1, OS)]
    base = [0]
    for p in phases:
        base.append(base[-1] + p[2])

    def kernel(x_hbm, k_hbm, v_hbm, wq_hbm, wo_hbm, wr_hbm, wg_hbm, wu_hbm, wd_hbm,
               o_ref,
               x_v, wr_v, wq_v, wo_v, wg_v, wu_v, wd_v, kbuf, vbuf,
               xn_s, q_s, s_s, m_s, o_s, h_s, y_s, a_s,
               sem_l, sem_h, sem_x):
        row = lax.broadcasted_iota(jnp.int32, (G, DH), 0)

        def mult(x, m):
            return x if isinstance(x, int) else pl.multiple_of(x, m)

        def l_dst(p, s):
            kind = phases[p][0]
            if kind == "Q":
                return wq_v.at[0, pl.ds(mult(s * RS, RS), RS), :]
            if kind == "O":
                return wo_v.at[pl.ds(mult(WO_TAIL0 + s * DH, DH), DH), :]
            dst = kbuf if kind == "K" else vbuf
            return dst.at[:, pl.ds(mult(s * RS, RS), RS), :]

        def l_wait(p, s):
            dst = l_dst(p, s)
            pltpu.make_async_copy(dst, dst, sem_l.at[(base[p] + s) % DEPTH]).wait()

        def l_start(p, s, c=True):
            kind, g, _ = phases[p]
            sem = sem_l.at[(base[p] + s) % DEPTH]
            if kind == "Q":
                src = wq_hbm.at[pl.ds(mult(s * RS, RS), RS), pl.ds(0, GC)]
                cond(c, lambda: pltpu.make_async_copy(src, l_dst(p, s), sem).start(priority=_LO))
                return
            if kind == "O":
                src = wo_hbm.at[pl.ds(mult(WO_TAIL0 + s * DH, DH), DH), :]
                cond(c, lambda: pltpu.make_async_copy(src, l_dst(p, s), sem).start(priority=_LO))
                return
            src, dst = (k_hbm, kbuf) if kind == "K" else (v_hbm, vbuf)

            def piece(r_src, r_dst, n):
                pltpu.make_async_copy(
                    src.at[0, pl.ds(g * G, G), pl.ds(SK - W + r_src, n), :],
                    dst.at[:, pl.ds(r_dst, n), :], sem).start(priority=_LO)

            def body():
                piece(mult(s * RS + SH, 8), mult(s * RS, RS), RS)

            def last():
                piece(W - RS + SH, W - RS, RS - SH)
                piece(0, W - SH, SH)

            if SH == 0:
                cond(c, body)
            else:
                cond(land(c, s < NS - 1), body)
                cond(land(c, s == NS - 1), last)

        def land(a, b):
            if isinstance(a, bool):
                return b if a else False
            if isinstance(b, bool):
                return a if b else False
            return jnp.logical_and(a, b)

        def cond(c, f):
            if isinstance(c, bool):
                if c:
                    f()
            else:
                pl.when(c)(f)

        def l_issue_ahead(p, s):
            n = phases[p][2]
            t = s + DEPTH
            if n > DEPTH:
                l_start(p, t, t < n)
            if p + 1 < len(phases):
                n1 = phases[p + 1][2]
                c = t >= n
                if n1 < DEPTH:
                    c = land(c, t - n < n1)
                l_start(p + 1, t - n, c)

        def rows_copy(src, dst, r, n, sem):
            return pltpu.make_async_copy(src.at[pl.ds(r, n), :], dst.at[pl.ds(r, n), :], sem)

        ffn = [(wg_hbm, wg_v), (wu_hbm, wu_v), (wd_hbm, wd_v)]

        def h_issue(p, s):
            kind, g, _ = phases[p]
            sem = sem_h.at[p]
            if kind == "Q":
                rows_copy(wo_hbm, wo_v, mult(s * 16, 16), 16, sem).start(priority=_HI)
            elif kind == "K" and g + 1 < NG:
                r = mult(s * 8, 8)
                pltpu.make_async_copy(
                    wq_hbm.at[pl.ds(r, 8), pl.ds((g + 1) * GC, GC)],
                    wq_v.at[g + 1, pl.ds(r, 8), :], sem).start(priority=_HI)
            elif kind == "K":
                rows_copy(wo_hbm, wo_v, mult(WO_Q0 + s * 24, 8), 24, sem).start(priority=_HI)
            elif kind == "V" and g + 1 < NG:
                src, dst = ffn[g]
                cond(s < F24, lambda: rows_copy(src, dst, mult(s * 24, 8), 24, sem).start(priority=_HI))
                cond(s >= F24, lambda: rows_copy(
                    src, dst, mult(F24 * 24 + (s - F24) * 16, 8), 16, sem).start(priority=_HI))
            elif kind == "V":
                half = NS // 2
                r = mult(WO_Q0 + WO_K + s * 24, 8)
                cond(s < half, lambda: rows_copy(wo_hbm, wo_v, r, 24, sem).start(priority=_HI))
                cond(s >= half, lambda: rows_copy(wo_hbm, wo_v, r, 24, sem_h.at[p + 1]).start(priority=_HI))

        def h_wait(p, ref):
            pltpu.make_async_copy(ref, ref, sem_h.at[p]).wait()

        def step(p, s):
            l_wait(p, s)
            h_issue(p, s)
            l_issue_ahead(p, s)

        def pick_rows(r):
            out = r[:, 0:DH]
            for i in range(1, G):
                out = jnp.where(row == i, r[:, i * DH:(i + 1) * DH], out)
            return out

        def qproj(g, k):
            r0 = mult(k * 128, 128)
            r = jnp.dot(xn_s[k].astype(_BF16), wq_v[g, pl.ds(r0, 128), :],
                        preferred_element_type=_F32)
            return pick_rows(r)

        def xn_full():
            return jnp.concatenate([xn_s[k] for k in range(D // 128)], axis=1)

        def woproj(h):
            r0 = mult(h * DH, DH)
            oh = jnp.broadcast_to(o_s[pl.ds(h, 1), :], (8, DH)).astype(_BF16)
            return jnp.dot(oh, wo_v[pl.ds(r0, DH), :], preferred_element_type=_F32)

        x_cp = pltpu.make_async_copy(x_hbm, x_v, sem_x.at[0])
        wr_cp = pltpu.make_async_copy(wr_hbm, wr_v, sem_x.at[1])
        x_cp.start(priority=_HI)
        for s in range(DEPTH):
            if s < QS:
                l_start(0, s)
            else:
                l_start(1, s - QS)
        wr_cp.start(priority=_HI)
        if FP > F:
            for _, dst in ffn:
                dst[pl.ds(F, FP - F), :] = jnp.zeros((FP - F, D), _BF16)

        x_cp.wait()
        x = x_v[0].astype(_F32)
        mu = jnp.mean(x, axis=-1, keepdims=True)
        xc = x - mu
        var = jnp.mean(xc * xc, axis=-1, keepdims=True)
        xn = (xc / jnp.sqrt(var + 1e-5)).astype(_BF16).astype(_F32)
        xn8 = jnp.broadcast_to(xn, (8, D))
        for k in range(D // 128):
            xn_s[k] = xn8[:, k * 128:(k + 1) * 128]

        q = None
        for t in range(QS // 2):
            step(0, 2 * t)
            step(0, 2 * t + 1)
            part = qproj(0, t)
            q = part if q is None else q + part
        q_s[...] = q

        carry_acc = None
        for g in range(NG):
            pk, pv = 1 + 2 * g, 2 + 2 * g

            def k_extra(t, g=g, pk=pk):
                if g == 0:
                    return
                idx = t - 1
                src = ffn[g - 1][1]

                @pl.when(t == 1)
                def _():
                    h_wait(pk - 1, src.at[pl.ds(0, F), :])

                @pl.when(jnp.logical_and(t >= 1, t <= FT))
                def _():
                    r0 = pl.multiple_of(idx * 128, 128)
                    w = src[pl.ds(r0, 128), :]
                    if g == 1:
                        h_s[idx] = lax.dot_general(xn_full().astype(_BF16), w, _NT,
                                                   preferred_element_type=_F32)
                    elif g == 2:
                        up = lax.dot_general(xn_full().astype(_BF16), w, _NT,
                                             preferred_element_type=_F32)
                        gt = h_s[idx]
                        h_s[idx] = gt * jax.nn.sigmoid(gt) * up
                    else:
                        y_s[...] += jnp.dot(h_s[idx].astype(_BF16), w, preferred_element_type=_F32)

                if g == NG - 1:
                    @pl.when(t == 0)
                    def _():
                        y_s[...] = jnp.zeros((8, D), _F32)

                    @pl.when(t == FT + 1)
                    def _():
                        wr_cp.wait()
                        xf = xn_full()
                        r = jnp.sum(xf * wr_v[...].astype(_F32).reshape(1, D), axis=-1, keepdims=True)
                        z = xf + y_s[...] * jax.nn.sigmoid(r)
                        y_s[...] = z * jax.nn.sigmoid(z)

            qb = q_s[...].astype(_BF16)

            def k_body(t, m, g=g, pk=pk, qb=qb, k_extra=k_extra):
                step(pk, 2 * t)
                k_extra(t)
                step(pk, 2 * t + 1)
                r0 = pl.multiple_of(t * 128, 128)
                kt = kbuf[:, pl.ds(r0, 128), :].reshape(G * 128, DH)
                s = pick_rows(lax.dot_general(qb, kt, _NT, preferred_element_type=_F32))
                s_s[t] = s
                return jnp.maximum(m, s)

            m = lax.fori_loop(0, NT, k_body, jnp.full((G, DH), -jnp.inf, _F32))
            m_s[...] = m

            def v_extra(t, g=g, pv=pv):
                @pl.when(t == 0)
                def _():
                    m_s[...] = jnp.broadcast_to(
                        jnp.max(m_s[...], axis=-1, keepdims=True), (G, DH))

                if g + 1 < NG:
                    @pl.when(t == 1)
                    def _():
                        h_wait(pv - 1, wq_v.at[g + 1])
                        q_s[...] = jnp.zeros((G, DH), _F32)

                    @pl.when(jnp.logical_and(t >= 1, t <= D // 128))
                    def _():
                        q_s[...] += qproj(g + 1, t - 1)
                else:
                    n1 = (WO_Q0 + WO_K) // DH
                    n2 = (WO_Q0 + WO_K + WO_V // 2) // DH
                    t2 = NT // 2 + 1

                    @pl.when(t == 1)
                    def _():
                        h_wait(0, wo_v.at[pl.ds(0, WO_Q0), :])
                        h_wait(pv - 1, wo_v.at[pl.ds(WO_Q0, WO_K), :])
                        a_s[...] = jnp.zeros((8, D), _F32)

                    @pl.when(t == t2)
                    def _():
                        h_wait(pv, wo_v.at[pl.ds(WO_Q0 + WO_K, WO_V // 2), :])

                    assert n1 + 1 <= t2
                    @pl.when(jnp.logical_or(jnp.logical_and(t >= 1, t <= n1),
                                            jnp.logical_and(t >= t2, t < t2 + n2 - n1)))
                    def _():
                        h = jnp.where(t <= n1, t - 1, t - t2 + n1)
                        a_s[...] += woproj(h)

            def v_body(t, carry, g=g, pv=pv, v_extra=v_extra):
                acc, l = carry
                step(pv, 2 * t)
                v_extra(t)
                step(pv, 2 * t + 1)
                r0 = pl.multiple_of(t * 128, 128)
                p = jnp.exp((s_s[t] - m_s[...]) * scale)
                vt = jnp.concatenate([vbuf[i, pl.ds(r0, 128), :] for i in range(G)], axis=1)
                r = jnp.dot(p.astype(_BF16), vt, preferred_element_type=_F32)
                return acc + pick_rows(r), l + p

            zero = jnp.zeros((G, DH), _F32)
            acc, l = lax.fori_loop(0, NT, v_body, (zero, zero))
            o_s[pl.ds(g * G, G), :] = acc / jnp.sum(l, axis=-1, keepdims=True)

        po = len(phases) - 1
        n2 = (WO_Q0 + WO_K + WO_V // 2) // DH
        n3 = WO_TAIL0 // DH
        a = a_s[...]
        for s in range(OS):
            l_wait(po, s)
            if s == 3:
                h_wait(po, wo_v.at[pl.ds(WO_Q0 + WO_K + WO_V // 2, WO_V // 2), :])
                for h in range(n2, n3):
                    a = a + woproj(h)
            a = a + woproj(n3 + s)
        res = x_v[0].astype(_F32) + a[0:1, :] * y_s[0:1, :]
        o_ref[0] = res.astype(o_ref.dtype)

    scratch = [
        pltpu.VMEM((1, 1, D), _BF16),
        pltpu.VMEM((D,), _BF16),
        pltpu.VMEM((NG, D, GC), _BF16),
        pltpu.VMEM((H * DH, D), _BF16),
        pltpu.VMEM((FP, D), _BF16),
        pltpu.VMEM((FP, D), _BF16),
        pltpu.VMEM((FP, D), _BF16),
        pltpu.VMEM((G, W, DH), _BF16),
        pltpu.VMEM((G, W, DH), _BF16),
        pltpu.VMEM((D // 128, 8, 128), _F32),
        pltpu.VMEM((G, DH), _F32),
        pltpu.VMEM((NT, G, 128), _F32),
        pltpu.VMEM((G, DH), _F32),
        pltpu.VMEM((H, DH), _F32),
        pltpu.VMEM((FT, 8, 128), _F32),
        pltpu.VMEM((8, D), _F32),
        pltpu.VMEM((8, D), _F32),
        pltpu.SemaphoreType.DMA((DEPTH,)),
        pltpu.SemaphoreType.DMA((len(phases),)),
        pltpu.SemaphoreType.DMA((2,)),
    ]
    return kernel, scratch


@jax.jit
def pallas_recurrent_scan__sliding_block_cached__moe_arch_mod__decode_kernel(
    A_x: jax.Array,
    A_k_cache: jax.Array,
    A_v_cache: jax.Array,
    A_wq: jax.Array,
    A_wo: jax.Array,
    B_x: jax.Array,
    B_w_r: jax.Array,
    B_w_gate: jax.Array,
    B_w_up: jax.Array,
    B_w_down: jax.Array,
):
    _, _, D = A_x.shape
    _, H, SK, DH = A_k_cache.shape
    W = min(4096, max(256, SK // 4))
    F = B_w_gate.shape[1]
    kernel, scratch = _make_kernel(D, H, SK, DH, W, F, DEPTH=8)
    hbm = pl.BlockSpec(memory_space=pltpu.MemorySpace.HBM)
    return pl.pallas_call(
        kernel,
        out_shape=jax.ShapeDtypeStruct(A_x.shape, A_x.dtype),
        in_specs=[hbm] * 9,
        out_specs=pl.BlockSpec(memory_space=pltpu.VMEM),
        scratch_shapes=scratch,
        compiler_params=pltpu.CompilerParams(
            vmem_limit_bytes=64 * 1024 * 1024,
            disable_bounds_checks=True,
            disable_semaphore_checks=True,
        ),
    )(A_x, A_k_cache, A_v_cache, A_wq, A_wo, B_w_r, B_w_gate.T, B_w_up.T, B_w_down)
```

```python
import jax
import jax.numpy as jnp
from jax import lax
import jax.experimental.pallas as pl
import jax.experimental.pallas.tpu as pltpu

_F32 = jnp.float32
_BF16 = jnp.bfloat16
_NT = (((1,), (1,)), ((), ()))

_HI = 0
_LO = 1

import contextlib
PROF = False
def scope(n):
    return jax.named_scope(n) if PROF else contextlib.nullcontext()

CFG = dict(SUB=4, DA=4, NO=4, NVPU=4, OHS=(8, 8, 8, 8), NL=3)


def _make_kernel(D, H, SK, DH, W, F, SUB, DA, NO, NVPU, OHS, NL):
    OH = sum(OHS)
    scale = DH ** -0.5
    G = 8
    NG = H // G
    TR = 128
    RS = TR // SUB
    SH = 16
    NT = W // TR
    DEPTH = SUB * DA
    GC = G * DH
    KD = D // 128
    FT = (F + 127) // 128
    FP = FT * 128
    assert NG == 4 and KD == DA and DEPTH & (DEPTH - 1) == 0

    if SUB == 2:
        S16, S40, S48, S32 = (8, 8), (24, 16), (24, 24), (16, 16)
    else:
        S16, S40, S48, S32 = (0, 8, 0, 8), (16, 8, 8, 8), (16, 8, 16, 8), (8, 8, 8, 8)
    F1 = NT * 40
    F2T = (F - F1) // 8
    assert F1 + F2T * 8 == F and 0 <= F2T <= NT
    WO0 = NO * DH
    E_Q = KD * 32
    E_K = NT * 16
    V3T = NT - 4
    WO_V = V3T * 32
    WO_K = NT * 48
    E_2 = H * DH - WO0 - E_Q - 2 * E_K - WO_K - WO_V
    assert 0 <= E_2 <= NT * 16 and E_2 % 16 == 0
    WO_E = E_Q + 2 * E_K + E_2
    assert WO_E % DH == 0 and WO_K % DH == 0
    HE = (WO0 + WO_E) // DH
    HK = (WO0 + WO_E + WO_K) // DH
    HL = (NG - 1) * G
    assert HE <= 2 * G and HK >= HL

    def kernel(x_hbm, k_hbm, v_hbm, wq_hbm, wo_hbm, wr_hbm, wg_hbm, wu_hbm, wd_hbm,
               o_ref,
               x_v, wr_v, wq_v, wo_v, wg_v, wu_v, wd_v, kbuf, vbuf,
               xn_s, q_s, s_s, m_s, il_s, o_s, h_s, y_s, a_s, ob_s,
               sem_l, sem_h, sem_e, sem_o, sem_x):
        row = lax.broadcasted_iota(jnp.int32, (G, DH), 0)
        ffn = [(wg_hbm, wg_v), (wu_hbm, wu_v), (wd_hbm, wd_v)]

        def mult(x, m):
            return x if isinstance(x, int) else pl.multiple_of(x, m)

        def cond(c, f):
            if isinstance(c, bool):
                if c:
                    f()
            else:
                pl.when(c)(f)

        def wait_all(ref, sem):
            pltpu.make_async_copy(ref, ref, sem).wait()

        def slot(t, u):
            return sem_l.at[(SUB * t + u) & (DEPTH - 1)]

        def l_wait(kind, t, u):
            r = pl.ds(mult(t * TR + u * RS, RS), RS)
            if kind == "Q":
                dst = wq_v.at[0, r, :]
            else:
                dst = (kbuf if kind == "K" else vbuf).at[:, r, :]
            wait_all(dst, slot(t, u))

        def q_start(t, u):
            r = pl.ds(t * TR + u * RS, RS)
            pltpu.make_async_copy(wq_hbm.at[r, pl.ds(0, GC)], wq_v.at[0, r, :],
                                  slot(t, u)).start(priority=_LO)

        def kv_piece(kind, g, r_src, r_dst, n, sem):
            src, dst = (k_hbm, kbuf) if kind == "K" else (v_hbm, vbuf)
            pltpu.make_async_copy(
                src.at[0, pl.ds(g * G, G), pl.ds(SK - W + r_src, n), :],
                dst.at[:, pl.ds(r_dst, n), :], sem).start(priority=_LO)

        def kv_start(kind, g, t, u):
            r = t * TR + u * RS
            kv_piece(kind, g, mult(r + SH, 8), mult(r, RS), RS, slot(t, u))

        def kv_start_wrapped(kind, g):
            sem = slot(NT - 1, SUB - 1)
            kv_piece(kind, g, W - RS + SH, W - RS, RS - SH, sem)
            kv_piece(kind, g, 0, W - SH, SH, sem)

        def rows_start(src, dst, r, n, sem, prio):
            pltpu.make_async_copy(src.at[pl.ds(r, n), :], dst.at[pl.ds(r, n), :],
                                  sem).start(priority=prio)

        def l_ahead(kind, g, t, u):
            ta = t + DA
            if u < SUB - 1:
                cond(ta < NT, lambda: kv_start(kind, g, ta, u))
            else:
                cond(ta < NT - 1, lambda: kv_start(kind, g, ta, u))
                cond(ta == NT - 1, lambda: kv_start_wrapped(kind, g))
            if kind == "K":
                cond(ta >= NT, lambda: kv_start("V", g, ta - NT, u))
            elif g + 1 < NG:
                cond(ta >= NT, lambda: kv_start("K", g + 1, ta - NT, u))
            elif u == 0:
                def tail():
                    for s in range(NO):
                        rows_start(wo_hbm, wo_v, s * DH, DH - (OH if s >= NO - NL else 0), sem_o.at[s], _LO)
                cond(ta == NT, tail)

        def stream(src, dst, sem, row0, sizes, t, u, tmax=None):
            n = sizes[u]
            if n == 0:
                return
            def go():
                r = row0 + t * sum(sizes) + sum(sizes[:u])
                rows_start(src, dst, mult(r, 8), n, sem, _HI)
            cond(True if tmax is None else t < tmax, go)

        def h_issue(kind, g, t, u):
            if kind == "Q":
                stream(wo_hbm, wo_v, sem_e.at[0], WO0, S32, t, u)
            elif kind == "K" and g + 1 < NG:
                nc = GC * 2 // SUB
                r = pl.ds(mult(t * 16 + (u * 2 // SUB) * 8, 8), 8)
                c0 = (u * nc) % GC
                pltpu.make_async_copy(
                    wq_hbm.at[r, pl.ds((g + 1) * GC + c0, nc)],
                    wq_v.at[g + 1, r, pl.ds(c0, nc)], sem_h.at[2 * g]).start(priority=_HI)
                stream(wo_hbm, wo_v, sem_e.at[0], WO0 + E_Q + g * E_K, S16, t, u,
                       None if g < 2 else E_2 // 16)
            elif kind == "K":
                stream(wo_hbm, wo_v, sem_h.at[2 * g], WO0 + WO_E, S48, t, u)
            elif g + 1 < NG:
                src, dst = ffn[g]
                stream(src, dst, sem_h.at[2 * g + 1], 0, S40, t, u)
                if u == SUB - 1:
                    stream(src, dst, sem_h.at[2 * g + 1], F1, (0,) * u + (8,), t, u, F2T)
            else:
                stream(wo_hbm, wo_v, sem_h.at[2 * g + 1], WO0 + WO_E + WO_K, S32, t, u, V3T)
                n = OHS[u]
                if n:
                    def late():
                        s = t - V3T + (NO - NL)
                        r = s * DH + DH - OH + sum(OHS[:u])
                        rows_start(wo_hbm, wo_v, mult(r, 8), n, sem_o.at[s], _HI)
                    cond(jnp.logical_and(t >= V3T, t < V3T + NL), late)

        def step(kind, g, t, u):
            l_wait(kind, t, u)
            h_issue(kind, g, t, u)
            if kind == "Q":
                kv_start("K", 0, t, u)
            else:
                l_ahead(kind, g, t, u)

        def pick_rows(r):
            out = r[:, 0:DH]
            for i in range(1, G):
                out = jnp.where(row == i, r[:, i * DH:(i + 1) * DH], out)
            return out

        def qproj(g, k):
            r = jnp.dot(xn_s[k].astype(_BF16), wq_v[g, pl.ds(mult(k * 128, 128), 128), :],
                        preferred_element_type=_F32)
            return pick_rows(r)

        def xn_full():
            return jnp.concatenate([xn_s[k] for k in range(KD)], axis=1)

        def woproj(h):
            oh = jnp.broadcast_to(o_s[pl.ds(h, 1), :], (8, DH)).astype(_BF16)
            return jnp.dot(oh, wo_v[pl.ds(mult(h * DH, DH), DH), :],
                           preferred_element_type=_F32)

        def between(t, lo, hi):
            return jnp.logical_and(t >= lo, t < hi)

        x_cp = pltpu.make_async_copy(x_hbm, x_v, sem_x.at[0])
        wr_cp = pltpu.make_async_copy(wr_hbm, wr_v, sem_x.at[1])
        x_cp.start(priority=_HI)
        for t in range(KD):
            for u in range(SUB):
                q_start(t, u)
        wr_cp.start(priority=_HI)
        if FP > F:
            for _, dst in ffn:
                dst[pl.ds(F, FP - F), :] = jnp.zeros((FP - F, D), _BF16)
        y_s[...] = jnp.zeros((8, D), _F32)
        a_s[...] = jnp.zeros((8, D), _F32)

        x_cp.wait()
        x = x_v[0].astype(_F32)
        mu = jnp.mean(x, axis=-1, keepdims=True)
        xc = x - mu
        var = jnp.mean(xc * xc, axis=-1, keepdims=True)
        xn = (xc / jnp.sqrt(var + 1e-5)).astype(_BF16).astype(_F32)
        xn8 = jnp.broadcast_to(xn, (8, D))
        for k in range(KD):
            xn_s[k] = xn8[:, k * 128:(k + 1) * 128]

        q = None
        for t in range(KD):
            for u in range(SUB):
                step("Q", 0, t, u)
            part = qproj(0, t)
            q = part if q is None else q + part
        with scope("q0done"):
            q_s[...] = q

        for g in range(NG):
            def k_extra(t, g=g):
                if g == 0:
                    return
                w_v = ffn[g - 1][1]
                T0 = 2

                @pl.when(t == T0)
                def _():
                    wait_all(w_v.at[pl.ds(0, F), :], sem_h.at[2 * g - 1])

                @pl.when(between(t, T0, T0 + FT))
                def _():
                    idx = t - T0
                    w = w_v[pl.ds(pl.multiple_of(idx * 128, 128), 128), :]
                    if g == 1:
                        h_s[idx] = lax.dot_general(xn_full().astype(_BF16), w, _NT,
                                                   preferred_element_type=_F32)
                    elif g == 2:
                        up = lax.dot_general(xn_full().astype(_BF16), w, _NT,
                                             preferred_element_type=_F32)
                        gt = h_s[idx]
                        h_s[idx] = gt * jax.nn.sigmoid(gt) * up
                    else:
                        y_s[...] += jnp.dot(h_s[idx].astype(_BF16), w, preferred_element_type=_F32)

                T1 = T0 + FT
                if g == 1 and NVPU:
                    @pl.when(between(t, T1, T1 + NVPU))
                    def _():
                        i = t - T1
                        oh = o_s[pl.ds(NO - NVPU + i, 1), :].astype(_BF16).astype(_F32)
                        ob_s[i] = jnp.transpose(jnp.broadcast_to(oh, (DH, DH)))

                if g == NG - 1:
                    @pl.when(t == T1)
                    def _():
                        wr_cp.wait()
                        xf = xn_full()
                        r = jnp.sum(xf * wr_v[...].astype(_F32).reshape(1, D), axis=-1, keepdims=True)
                        z = xf + y_s[...] * jax.nn.sigmoid(r)
                        y_s[...] = z * jax.nn.sigmoid(z)
                        wait_all(wo_v.at[pl.ds(WO0, WO_E), :], sem_e.at[0])

                    @pl.when(between(t, T1 + 1, T1 + 1 + HE - NO))
                    def _():
                        a_s[...] += woproj(t - (T1 + 1) + NO)

            qb = q_s[...].astype(_BF16)

            def k_body(t, m, g=g, qb=qb, k_extra=k_extra):
                step("K", g, t, 0)
                k_extra(t)
                for u in range(1, SUB):
                    step("K", g, t, u)
                kt = kbuf[:, pl.ds(pl.multiple_of(t * TR, TR), TR), :].reshape(G * TR, DH)
                s = pick_rows(lax.dot_general(qb, kt, _NT, preferred_element_type=_F32))
                s_s[t] = s
                return jnp.maximum(m, s)

            with scope("kloop%d" % g):
                m_s[...] = lax.fori_loop(0, NT, k_body, jnp.full((G, DH), -jnp.inf, _F32))

            def v_extra(t, g=g):
                @pl.when(t == 0)
                def _():
                    m_s[...] = jnp.broadcast_to(
                        jnp.max(m_s[...], axis=-1, keepdims=True), (G, DH))

                @pl.when(t == 1)
                def _():
                    p = jnp.exp((s_s[...] - m_s[...][None]) * scale)
                    l = jnp.sum(jnp.sum(p, axis=0), axis=-1, keepdims=True)
                    il_s[...] = jnp.broadcast_to(1.0 / l, (G, DH))

                T0 = 2
                if g + 1 < NG:
                    @pl.when(t == T0)
                    def _():
                        wait_all(wq_v.at[g + 1], sem_h.at[2 * g])
                        q_s[...] = jnp.zeros((G, DH), _F32)

                    @pl.when(between(t, T0, T0 + KD))
                    def _():
                        q_s[...] += qproj(g + 1, t - T0)
                else:
                    @pl.when(t == T0)
                    def _():
                        wait_all(wo_v.at[pl.ds(WO0 + WO_E, WO_K), :], sem_h.at[2 * g])

                    @pl.when(between(t, T0, T0 + HL - HE))
                    def _():
                        a_s[...] += woproj(t - T0 + HE)

            def v_body(t, acc, g=g, v_extra=v_extra):
                step("V", g, t, 0)
                v_extra(t)
                for u in range(1, SUB):
                    step("V", g, t, u)
                r0 = pl.multiple_of(t * TR, TR)
                p = jnp.exp((s_s[t] - m_s[...]) * scale)
                vt = jnp.concatenate([vbuf[i, pl.ds(r0, TR), :] for i in range(G)], axis=1)
                r = jnp.dot(p.astype(_BF16), vt, preferred_element_type=_F32)
                return acc + pick_rows(r)

            with scope("vloop%d" % g):
                acc = lax.fori_loop(0, NT, v_body, jnp.zeros((G, DH), _F32))
            o_s[pl.ds(g * G, G), :] = acc * il_s[...]

        with scope("hwait"):
            wait_all(wo_v.at[pl.ds(WO0 + WO_E + WO_K, WO_V), :], sem_h.at[2 * NG - 1])
        for s in range(NO - NVPU):
            with scope("owait%d" % s):
                wait_all(wo_v.at[pl.ds(s * DH, DH), :], sem_o.at[s])
        a = a_s[...]
        for h in list(range(HL, H)) + list(range(NO - NVPU)):
            a = a + woproj(h)
        a = a[0:1, :]
        part = None
        for i in range(NVPU):
            s = NO - NVPU + i
            with scope("owait%d" % s):
                wait_all(wo_v.at[pl.ds(s * DH, DH), :], sem_o.at[s])
            w = wo_v[pl.ds(s * DH, DH), :].astype(_F32)
            ob = ob_s[i]
            pr = w * jnp.concatenate([ob] * KD, axis=1)
            pr = jnp.sum(pr.reshape(DH // 8, 8, D), axis=0)
            part = pr if part is None else part + pr
        if part is not None:
            a = a + jnp.sum(part, axis=0, keepdims=True)
        res = x_v[0].astype(_F32) + a * y_s[0:1, :]
        with scope("store"):
            o_ref[0] = res.astype(o_ref.dtype)

    scratch = [
        pltpu.VMEM((1, 1, D), _BF16),
        pltpu.VMEM((D,), _BF16),
        pltpu.VMEM((NG, D, GC), _BF16),
        pltpu.VMEM((H * DH, D), _BF16),
        pltpu.VMEM((FP, D), _BF16),
        pltpu.VMEM((FP, D), _BF16),
        pltpu.VMEM((FP, D), _BF16),
        pltpu.VMEM((G, W, DH), _BF16),
        pltpu.VMEM((G, W, DH), _BF16),
        pltpu.VMEM((KD, 8, 128), _F32),
        pltpu.VMEM((G, DH), _F32),
        pltpu.VMEM((NT, G, 128), _F32),
        pltpu.VMEM((G, DH), _F32),
        pltpu.VMEM((G, DH), _F32),
        pltpu.VMEM((H, DH), _F32),
        pltpu.VMEM((FT, 8, 128), _F32),
        pltpu.VMEM((8, D), _F32),
        pltpu.VMEM((8, D), _F32),
        pltpu.VMEM((max(NVPU, 1), DH, DH), _F32),
        pltpu.SemaphoreType.DMA((DEPTH,)),
        pltpu.SemaphoreType.DMA((2 * NG,)),
        pltpu.SemaphoreType.DMA((1,)),
        pltpu.SemaphoreType.DMA((NO,)),
        pltpu.SemaphoreType.DMA((2,)),
    ]
    return kernel, scratch


@jax.jit
def pallas_recurrent_scan__sliding_block_cached__moe_arch_mod__decode_kernel(
    A_x: jax.Array,
    A_k_cache: jax.Array,
    A_v_cache: jax.Array,
    A_wq: jax.Array,
    A_wo: jax.Array,
    B_x: jax.Array,
    B_w_r: jax.Array,
    B_w_gate: jax.Array,
    B_w_up: jax.Array,
    B_w_down: jax.Array,
):
    _, _, D = A_x.shape
    _, H, SK, DH = A_k_cache.shape
    W = min(4096, max(256, SK // 4))
    F = B_w_gate.shape[1]
    kernel, scratch = _make_kernel(D, H, SK, DH, W, F, **CFG)
    hbm = pl.BlockSpec(memory_space=pltpu.MemorySpace.HBM)
    return pl.pallas_call(
        kernel,
        out_shape=jax.ShapeDtypeStruct(A_x.shape, A_x.dtype),
        in_specs=[hbm] * 9,
        out_specs=pl.BlockSpec(memory_space=pltpu.VMEM),
        scratch_shapes=scratch,
        compiler_params=pltpu.CompilerParams(
            vmem_limit_bytes=64 * 1024 * 1024,
            disable_bounds_checks=True,
            disable_semaphore_checks=True,
        ),
    )(A_x, A_k_cache, A_v_cache, A_wq, A_wo, B_w_r, B_w_gate.T, B_w_up.T, B_w_down)
```

```python
import jax
import jax.numpy as jnp
from jax import lax
import jax.experimental.pallas as pl
import jax.experimental.pallas.tpu as pltpu

_F32 = jnp.float32
_BF16 = jnp.bfloat16
_NT = (((1,), (1,)), ((), ()))


def _rnd(v):
    return v.astype(_BF16).astype(_F32)


_HI = 0
_LO = 1

import contextlib
PROF = False
def scope(n):
    return jax.named_scope(n) if PROF else contextlib.nullcontext()

CFG = dict(RSZ=(40, 40, 24, 24), SH=8, DA=4, NO=4, NVPU=4, NL=3, XOFF=0,
           QP=((0, 128, 0, 256), (0, 128, 256, 256), (0, 128, 512, 256), (0, 128, 768, 256)))


def _make_kernel(D, H, SK, DH, W, F, RSZ, SH, DA, NO, NVPU, NL, XOFF, QP):
    SUB = len(RSZ)
    scale = DH ** -0.5
    G = 8
    NG = H // G
    TR = 128
    assert sum(RSZ) == TR and RSZ[-1] > SH
    ROFF = [sum(RSZ[:u]) for u in range(SUB)]
    NT = W // TR
    DEPTH = SUB * DA
    GC = G * DH
    KD = D // 128
    FT = (F + 127) // 128
    FP = FT * 128
    assert NG == 4 and KD == DA and DA & (DA - 1) == 0

    if SUB == 2:
        S16, S40, S48, S32 = (8, 8), (24, 16), (24, 24), (16, 16)
        WQP = ((0, 0, GC), (8, 0, GC))
    elif SUB == 3:
        S16, S40, S48, S32 = (0, 8, 8), (16, 16, 8), (16, 16, 16), (16, 8, 8)
        WQP = ((0, 0, GC), (8, 0, GC // 2), (8, GC // 2, GC // 2))
    else:
        S16, S40, S48, S32 = (0, 8, 0, 8), (16, 8, 8, 8), (16, 8, 16, 8), (8, 8, 8, 8)
        WQP = ((0, 0, GC // 2), (0, GC // 2, GC // 2), (8, 0, GC // 2), (8, GC // 2, GC // 2))
    OHS = S32
    OH = sum(OHS)
    F1 = NT * 40
    F2T = (F - F1) // 8
    assert F1 + F2T * 8 == F and 0 <= F2T <= NT
    WO0 = NO * DH
    E_Q = KD * 32
    E_K = NT * 16
    V3T = NT - 4
    WO_V = V3T * 32
    WO_K = NT * 48
    E_2 = H * DH - WO0 - E_Q - 2 * E_K - WO_K - WO_V
    assert 0 <= E_2 <= NT * 16 and E_2 % 16 == 0
    WO_E = E_Q + 2 * E_K + E_2
    assert WO_E % DH == 0 and WO_K % DH == 0
    HE = (WO0 + WO_E) // DH
    HK = (WO0 + WO_E + WO_K) // DH
    HL = (NG - 1) * G
    assert HE <= 2 * G and HK >= HL

    def kernel(x_hbm, k_hbm, v_hbm, wq_hbm, wo_hbm, wr_hbm, wg_hbm, wu_hbm, wd_hbm,
               o_ref,
               x_v, wr_v, wq_v, wo_v, wg_v, wu_v, wd_v, kbuf, vbuf,
               xn_s, q_s, s_s, m_s, il_s, o_s, h_s, y_s, a_s, ob_s,
               sem_l, sem_h, sem_e, sem_o, sem_x):
        row = lax.broadcasted_iota(jnp.int32, (G, DH), 0)
        ffn = [(wg_hbm, wg_v), (wu_hbm, wu_v), (wd_hbm, wd_v)]

        def mult(x, m):
            return x if isinstance(x, int) else pl.multiple_of(x, m)

        def cond(c, f):
            if isinstance(c, bool):
                if c:
                    f()
            else:
                pl.when(c)(f)

        def wait_all(ref, sem):
            pltpu.make_async_copy(ref, ref, sem).wait()

        def slot(t, u):
            return sem_l.at[(t & (DA - 1)) * SUB + u]

        def l_wait(kind, t, u):
            if kind == "Q":
                r0, nr, c0, nc = QP[u]
                dst = wq_v.at[0, pl.ds(t * TR + r0, nr), pl.ds(c0, nc)]
            else:
                r = pl.ds(mult(t * TR + ROFF[u], 8), RSZ[u])
                dst = (kbuf if kind == "K" else vbuf).at[:, r, :]
            wait_all(dst, slot(t, u))

        def q_start(t, u):
            r0, nr, c0, nc = QP[u]
            r, c = pl.ds(t * TR + r0, nr), pl.ds(c0, nc)
            pltpu.make_async_copy(wq_hbm.at[r, c], wq_v.at[0, r, c],
                                  slot(t, u)).start(priority=_LO)

        def kv_piece(kind, g, r_src, r_dst, n, sem):
            src, dst = (k_hbm, kbuf) if kind == "K" else (v_hbm, vbuf)
            pltpu.make_async_copy(
                src.at[0, pl.ds(g * G, G), pl.ds(SK - W - XOFF + r_src, n), :],
                dst.at[:, pl.ds(r_dst, n), :], sem).start(priority=_LO)

        def kv_start(kind, g, t, u):
            r = t * TR + ROFF[u]
            kv_piece(kind, g, mult(r + SH, 8), mult(r, 8), RSZ[u], slot(t, u))

        def kv_start_wrapped(kind, g):
            sem = slot(NT - 1, SUB - 1)
            n = RSZ[-1]
            kv_piece(kind, g, W - n + SH, W - n, n - SH, sem)
            kv_piece(kind, g, 0, W - SH, SH, sem)

        def rows_start(src, dst, r, n, sem, prio):
            pltpu.make_async_copy(src.at[pl.ds(r, n), :], dst.at[pl.ds(r, n), :],
                                  sem).start(priority=prio)

        def l_ahead(kind, g, t, u):
            ta = t + DA
            if u < SUB - 1:
                cond(ta < NT, lambda: kv_start(kind, g, ta, u))
            else:
                cond(ta < NT - 1, lambda: kv_start(kind, g, ta, u))
                cond(ta == NT - 1, lambda: kv_start_wrapped(kind, g))
            if kind == "K":
                cond(ta >= NT, lambda: kv_start("V", g, ta - NT, u))
            elif g + 1 < NG:
                cond(ta >= NT, lambda: kv_start("K", g + 1, ta - NT, u))
            elif u == 0:
                def tail():
                    for s in range(NO):
                        rows_start(wo_hbm, wo_v, s * DH, DH - (OH if s >= NO - NL else 0), sem_o.at[s], _LO)
                cond(ta == NT, tail)

        def stream(src, dst, sem, row0, sizes, t, u, tmax=None):
            n = sizes[u]
            if n == 0:
                return
            def go():
                r = row0 + t * sum(sizes) + sum(sizes[:u])
                rows_start(src, dst, mult(r, 8), n, sem, _HI)
            cond(True if tmax is None else t < tmax, go)

        def h_issue(kind, g, t, u):
            if kind == "Q":
                stream(wo_hbm, wo_v, sem_e.at[0], WO0, S32, t, u)
            elif kind == "K" and g + 1 < NG:
                r0, c0, nc = WQP[u]
                r = pl.ds(mult(t * 16 + r0, 8), 8)
                pltpu.make_async_copy(
                    wq_hbm.at[r, pl.ds((g + 1) * GC + c0, nc)],
                    wq_v.at[g + 1, r, pl.ds(c0, nc)], sem_h.at[2 * g]).start(priority=_HI)
                stream(wo_hbm, wo_v, sem_e.at[0], WO0 + E_Q + g * E_K, S16, t, u,
                       None if g < 2 else E_2 // 16)
            elif kind == "K":
                stream(wo_hbm, wo_v, sem_h.at[2 * g], WO0 + WO_E, S48, t, u)
            elif g + 1 < NG:
                src, dst = ffn[g]
                stream(src, dst, sem_h.at[2 * g + 1], 0, S40, t, u)
                if u == SUB - 1:
                    stream(src, dst, sem_h.at[2 * g + 1], F1, (0,) * u + (8,), t, u, F2T)
            else:
                stream(wo_hbm, wo_v, sem_h.at[2 * g + 1], WO0 + WO_E + WO_K, S32, t, u, V3T)
                n = OHS[u]
                if n:
                    def late():
                        s = t - V3T + (NO - NL)
                        r = s * DH + DH - OH + sum(OHS[:u])
                        rows_start(wo_hbm, wo_v, mult(r, 8), n, sem_o.at[s], _HI)
                    cond(jnp.logical_and(t >= V3T, t < V3T + NL), late)

        def step(kind, g, t, u):
            l_wait(kind, t, u)
            h_issue(kind, g, t, u)
            if kind == "Q":
                kv_start("K", 0, t, u)
            else:
                l_ahead(kind, g, t, u)

        def pick_rows(r):
            out = r[:, 0:DH]
            for i in range(1, G):
                out = jnp.where(row == i, r[:, i * DH:(i + 1) * DH], out)
            return out

        def qproj(g, k):
            r = jnp.dot(xn_s[k].astype(_BF16), wq_v[g, pl.ds(mult(k * 128, 128), 128), :],
                        preferred_element_type=_F32)
            return pick_rows(r)

        def xn_full():
            return jnp.concatenate([xn_s[k] for k in range(KD)], axis=1)

        def woproj(h):
            oh = jnp.broadcast_to(o_s[pl.ds(h, 1), :], (8, DH)).astype(_BF16)
            return jnp.dot(oh, wo_v[pl.ds(mult(h * DH, DH), DH), :],
                           preferred_element_type=_F32)

        def between(t, lo, hi):
            return jnp.logical_and(t >= lo, t < hi)

        x_cp = pltpu.make_async_copy(x_hbm, x_v, sem_x.at[0])
        wr_cp = pltpu.make_async_copy(wr_hbm, wr_v, sem_x.at[1])
        x_cp.start(priority=_HI)
        for t in range(KD):
            for u in range(SUB):
                q_start(t, u)
        wr_cp.start(priority=_HI)
        if FP > F:
            for _, dst in ffn:
                dst[pl.ds(F, FP - F), :] = jnp.zeros((FP - F, D), _BF16)
        y_s[...] = jnp.zeros((8, D), _F32)
        a_s[...] = jnp.zeros((8, D), _F32)

        with scope("xwait"):
            x_cp.wait()
        x = x_v[0].astype(_F32)
        mu = jnp.mean(x, axis=-1, keepdims=True)
        xc = x - mu
        var = jnp.mean(xc * xc, axis=-1, keepdims=True)
        den = _rnd(jnp.sqrt(_rnd(_rnd(var) + 1e-5)))
        xn = _rnd(_rnd(x - _rnd(mu)) / den)
        xn8 = jnp.broadcast_to(xn, (8, D))
        for k in range(KD):
            xn_s[k] = xn8[:, k * 128:(k + 1) * 128]

        q = None
        for t in range(KD):
            for u in range(SUB):
                with scope("q%d_%d" % (t, u)):
                    step("Q", 0, t, u)
            part = qproj(0, t)
            q = part if q is None else q + part
        with scope("q0done"):
            q_s[...] = q

        for g in range(NG):
            def k_extra(t, g=g):
                if g == 0:
                    return
                w_v = ffn[g - 1][1]
                T0 = 2

                @pl.when(t == T0)
                def _():
                    wait_all(w_v.at[pl.ds(0, F), :], sem_h.at[2 * g - 1])

                @pl.when(between(t, T0, T0 + FT))
                def _():
                    idx = t - T0
                    w = w_v[pl.ds(pl.multiple_of(idx * 128, 128), 128), :]
                    if g == 1:
                        h_s[idx] = lax.dot_general(xn_full().astype(_BF16), w, _NT,
                                                   preferred_element_type=_F32)
                    elif g == 2:
                        up = lax.dot_general(xn_full().astype(_BF16), w, _NT,
                                             preferred_element_type=_F32)
                        gt = _rnd(h_s[idx])
                        h_s[idx] = _rnd(gt * jax.nn.sigmoid(gt)) * _rnd(up)
                    else:
                        y_s[...] += jnp.dot(h_s[idx].astype(_BF16), w, preferred_element_type=_F32)

                T1 = T0 + FT
                if g == 1 and NVPU:
                    @pl.when(between(t, T1, T1 + NVPU))
                    def _():
                        i = t - T1
                        oh = _rnd(o_s[pl.ds(NO - NVPU + i, 1), :])
                        ob_s[i] = jnp.transpose(jnp.broadcast_to(oh, (DH, DH)))

                if g == NG - 1:
                    @pl.when(t == T1)
                    def _():
                        wr_cp.wait()
                        xf = xn_full()
                        r = jnp.sum(xf * wr_v[...].astype(_F32).reshape(1, D), axis=-1, keepdims=True)
                        r_sel = _rnd(jax.nn.sigmoid(_rnd(r)))
                        z = _rnd(xf + _rnd(_rnd(y_s[...]) * r_sel))
                        y_s[...] = _rnd(z * jax.nn.sigmoid(z))
                        wait_all(wo_v.at[pl.ds(WO0, WO_E), :], sem_e.at[0])

                    @pl.when(between(t, T1 + 1, T1 + 1 + HE - NO))
                    def _():
                        a_s[...] += woproj(t - (T1 + 1) + NO)

            qb = q_s[...].astype(_BF16)

            def k_body(t, m, g=g, qb=qb, k_extra=k_extra):
                step("K", g, t, 0)
                k_extra(t)
                for u in range(1, SUB):
                    step("K", g, t, u)
                kt = kbuf[:, pl.ds(pl.multiple_of(t * TR, TR), TR), :].reshape(G * TR, DH)
                s = pick_rows(lax.dot_general(qb, kt, _NT, preferred_element_type=_F32))
                s_s[t] = s
                return jnp.maximum(m, s)

            with scope("kloop%d" % g):
                m_s[...] = lax.fori_loop(0, NT, k_body, jnp.full((G, DH), -jnp.inf, _F32))

            def v_extra(t, g=g):
                @pl.when(t == 0)
                def _():
                    m_s[...] = jnp.broadcast_to(
                        jnp.max(m_s[...], axis=-1, keepdims=True), (G, DH))

                @pl.when(t == 1)
                def _():
                    p = jnp.exp((s_s[...] - m_s[...][None]) * scale)
                    l = jnp.sum(jnp.sum(p, axis=0), axis=-1, keepdims=True)
                    il_s[...] = jnp.broadcast_to(1.0 / l, (G, DH))

                T0 = 2
                if g + 1 < NG:
                    @pl.when(t == T0)
                    def _():
                        wait_all(wq_v.at[g + 1], sem_h.at[2 * g])
                        q_s[...] = jnp.zeros((G, DH), _F32)

                    @pl.when(between(t, T0, T0 + KD))
                    def _():
                        q_s[...] += qproj(g + 1, t - T0)
                else:
                    @pl.when(t == T0)
                    def _():
                        wait_all(wo_v.at[pl.ds(WO0 + WO_E, WO_K), :], sem_h.at[2 * g])

                    @pl.when(between(t, T0, T0 + HL - HE))
                    def _():
                        a_s[...] += woproj(t - T0 + HE)

            def v_body(t, acc, g=g, v_extra=v_extra):
                step("V", g, t, 0)
                v_extra(t)
                for u in range(1, SUB):
                    step("V", g, t, u)
                r0 = pl.multiple_of(t * TR, TR)
                p = jnp.exp((s_s[t] - m_s[...]) * scale)
                vt = jnp.concatenate([vbuf[i, pl.ds(r0, TR), :] for i in range(G)], axis=1)
                r = jnp.dot(p.astype(_BF16), vt, preferred_element_type=_F32)
                return acc + pick_rows(r)

            with scope("vloop%d" % g):
                acc = lax.fori_loop(0, NT, v_body, jnp.zeros((G, DH), _F32))
            o_s[pl.ds(g * G, G), :] = acc * il_s[...]

        with scope("hwait"):
            wait_all(wo_v.at[pl.ds(WO0 + WO_E + WO_K, WO_V), :], sem_h.at[2 * NG - 1])
        for s in range(NO - NVPU):
            with scope("owait%d" % s):
                wait_all(wo_v.at[pl.ds(s * DH, DH), :], sem_o.at[s])
        a = a_s[...]
        for h in list(range(HL, H)) + list(range(NO - NVPU)):
            a = a + woproj(h)
        a = a[0:1, :]
        part = None
        for i in range(NVPU):
            s = NO - NVPU + i
            with scope("owait%d" % s):
                wait_all(wo_v.at[pl.ds(s * DH, DH), :], sem_o.at[s])
            w = wo_v[pl.ds(s * DH, DH), :].astype(_F32)
            ob = ob_s[i]
            pr = w * jnp.concatenate([ob] * KD, axis=1)
            pr = jnp.sum(pr.reshape(DH // 8, 8, D), axis=0)
            part = pr if part is None else part + pr
        if part is not None:
            a = a + jnp.sum(part, axis=0, keepdims=True)
        res = x_v[0].astype(_F32) + _rnd(_rnd(a) * y_s[0:1, :])
        with scope("store"):
            o_ref[0] = res.astype(o_ref.dtype)

    scratch = [
        pltpu.VMEM((1, 1, D), _BF16),
        pltpu.VMEM((D,), _BF16),
        pltpu.VMEM((NG, D, GC), _BF16),
        pltpu.VMEM((H * DH, D), _BF16),
        pltpu.VMEM((FP, D), _BF16),
        pltpu.VMEM((FP, D), _BF16),
        pltpu.VMEM((FP, D), _BF16),
        pltpu.VMEM((G, W, DH), _BF16),
        pltpu.VMEM((G, W, DH), _BF16),
        pltpu.VMEM((KD, 8, 128), _F32),
        pltpu.VMEM((G, DH), _F32),
        pltpu.VMEM((NT, G, 128), _F32),
        pltpu.VMEM((G, DH), _F32),
        pltpu.VMEM((G, DH), _F32),
        pltpu.VMEM((H, DH), _F32),
        pltpu.VMEM((FT, 8, 128), _F32),
        pltpu.VMEM((8, D), _F32),
        pltpu.VMEM((8, D), _F32),
        pltpu.VMEM((max(NVPU, 1), DH, DH), _F32),
        pltpu.SemaphoreType.DMA((DEPTH,)),
        pltpu.SemaphoreType.DMA((2 * NG,)),
        pltpu.SemaphoreType.DMA((1,)),
        pltpu.SemaphoreType.DMA((NO,)),
        pltpu.SemaphoreType.DMA((2,)),
    ]
    return kernel, scratch


@jax.jit
def pallas_recurrent_scan__sliding_block_cached__moe_arch_mod__decode_kernel(
    A_x: jax.Array,
    A_k_cache: jax.Array,
    A_v_cache: jax.Array,
    A_wq: jax.Array,
    A_wo: jax.Array,
    B_x: jax.Array,
    B_w_r: jax.Array,
    B_w_gate: jax.Array,
    B_w_up: jax.Array,
    B_w_down: jax.Array,
):
    _, _, D = A_x.shape
    _, H, SK, DH = A_k_cache.shape
    W = min(4096, max(256, SK // 4))
    F = B_w_gate.shape[1]
    kernel, scratch = _make_kernel(D, H, SK, DH, W, F, **CFG)
    hbm = pl.BlockSpec(memory_space=pltpu.MemorySpace.HBM)
    return pl.pallas_call(
        kernel,
        out_shape=jax.ShapeDtypeStruct(A_x.shape, A_x.dtype),
        in_specs=[hbm] * 9,
        out_specs=pl.BlockSpec(memory_space=pltpu.VMEM),
        scratch_shapes=scratch,
        compiler_params=pltpu.CompilerParams(
            vmem_limit_bytes=64 * 1024 * 1024,
            disable_bounds_checks=True,
            disable_semaphore_checks=True,
        ),
    )(A_x, A_k_cache, A_v_cache, A_wq, A_wo, B_w_r, B_w_gate.T, B_w_up.T, B_w_down)
```

```python
import jax
import jax.numpy as jnp
from jax import lax
import jax.experimental.pallas as pl
import jax.experimental.pallas.tpu as pltpu

_F32 = jnp.float32
_BF16 = jnp.bfloat16
_NT = (((1,), (1,)), ((), ()))

_HI = 0
_LO = 1


def _rnd(v):
    return v.astype(_BF16).astype(_F32)


def _make_kernel(D, H, SK, DH, W, F):
    scale = DH ** -0.5
    G = 8
    NG = H // G
    TR = 128
    NT = W // TR
    RSZ = (40, 40, 24, 24)
    SUB = len(RSZ)
    ROFF = [sum(RSZ[:u]) for u in range(SUB)]
    SH = 8
    DA = 4
    GC = G * DH
    QC = GC // SUB
    KD = D // 128
    FT = (F + 127) // 128
    FP = FT * 128
    assert NG == 4 and KD == DA and sum(RSZ) == TR and DH == 128

    S16, S32, S40, S48 = (0, 8, 0, 8), (8, 8, 8, 8), (16, 8, 8, 8), (16, 8, 16, 8)
    F1 = NT * 40
    F2T = (F - F1) // 8
    assert F1 + F2T * 8 == F and 0 <= F2T <= NT

    NO = 4
    WO0 = NO * DH
    NL = 3
    TBLK = (NL * 32, 128, 128, 128, 32)
    TOFF = [sum(TBLK[:i]) for i in range(len(TBLK))]
    TREG = ((1,), (0, 2), (3,), (4,))
    E_Q = KD * 32
    E_K = NT * 16
    WO_E = E_Q + 2 * E_K
    WO_K = NT * 48
    V3T = NT - 4
    WO_V = V3T * 32
    assert sum(TBLK) == WO0 and WO0 + WO_E + WO_K + WO_V == H * DH
    assert WO_E % DH == 0 and WO_K % DH == 0
    HE = (WO0 + WO_E) // DH
    HL = (NG - 1) * G
    assert HE <= 2 * G and (WO0 + WO_E + WO_K) // DH >= HL

    def kernel(x_hbm, k_hbm, v_hbm, wq_hbm, wo_hbm, wr_hbm, wg_hbm, wu_hbm, wd_hbm,
               o_ref,
               x_v, wr_v, wq_v, wo_v, wg_v, wu_v, wd_v, kbuf, vbuf,
               xn_s, q_s, s_s, m_s, il_s, o_s, h_s, y_s, a_s, ob_s,
               sem_l, sem_h, sem_e, sem_o, sem_x):
        row = lax.broadcasted_iota(jnp.int32, (G, DH), 0)
        ffn = [(wg_hbm, wg_v), (wu_hbm, wu_v), (wd_hbm, wd_v)]

        def mult(x, m):
            return x if isinstance(x, int) else pl.multiple_of(x, m)

        def cond(c, f):
            if isinstance(c, bool):
                if c:
                    f()
            else:
                pl.when(c)(f)

        def between(t, lo, hi):
            return jnp.logical_and(t >= lo, t < hi)

        def wait_all(ref, sem):
            pltpu.make_async_copy(ref, ref, sem).wait()

        def rows_start(src, dst, r, n, sem, prio):
            pltpu.make_async_copy(src.at[pl.ds(r, n), :], dst.at[pl.ds(r, n), :],
                                  sem).start(priority=prio)

        def slot(t, u):
            return sem_l.at[(t & (DA - 1)) * SUB + u]

        def l_wait(kind, t, u):
            if kind == "Q":
                dst = wq_v.at[0, pl.ds(t * TR, TR), pl.ds(u * QC, QC)]
            else:
                r = pl.ds(mult(t * TR + ROFF[u], 8), RSZ[u])
                dst = (kbuf if kind == "K" else vbuf).at[:, r, :]
            wait_all(dst, slot(t, u))

        def q_start(t, u):
            r, c = pl.ds(t * TR, TR), pl.ds(u * QC, QC)
            pltpu.make_async_copy(wq_hbm.at[r, c], wq_v.at[0, r, c],
                                  slot(t, u)).start(priority=_LO)

        def kv_piece(kind, g, r_src, r_dst, n, sem):
            src, dst = (k_hbm, kbuf) if kind == "K" else (v_hbm, vbuf)
            pltpu.make_async_copy(
                src.at[0, pl.ds(g * G, G), pl.ds(SK - W + r_src, n), :],
                dst.at[:, pl.ds(r_dst, n), :], sem).start(priority=_LO)

        def kv_start(kind, g, t, u):
            r = t * TR + ROFF[u]
            kv_piece(kind, g, mult(r + SH, 8), mult(r, 8), RSZ[u], slot(t, u))

        def kv_start_wrapped(kind, g):
            n, sem = RSZ[-1], slot(NT - 1, SUB - 1)
            kv_piece(kind, g, W - n + SH, W - n, n - SH, sem)
            kv_piece(kind, g, 0, W - SH, SH, sem)

        def tail_start():
            for s in range(1, len(TBLK)):
                rows_start(wo_hbm, wo_v, TOFF[s], TBLK[s], sem_o.at[s], _LO)

        def l_ahead(kind, g, t, u):
            ta = t + DA
            if u < SUB - 1:
                cond(ta < NT, lambda: kv_start(kind, g, ta, u))
            else:
                cond(ta < NT - 1, lambda: kv_start(kind, g, ta, u))
                cond(ta == NT - 1, lambda: kv_start_wrapped(kind, g))
            if kind == "K":
                cond(ta >= NT, lambda: kv_start("V", g, ta - NT, u))
            elif g + 1 < NG:
                cond(ta >= NT, lambda: kv_start("K", g + 1, ta - NT, u))
            elif u == 0:
                cond(ta == NT, tail_start)

        def stream(src, dst, sem, row0, sizes, t, u, active=True):
            if sizes[u]:
                def go():
                    r = row0 + t * sum(sizes) + sum(sizes[:u])
                    rows_start(src, dst, mult(r, 8), sizes[u], sem, _HI)
                cond(active, go)

        def h_issue(kind, g, t, u):
            if kind == "Q":
                stream(wo_hbm, wo_v, sem_e.at[0], WO0, S32, t, u)
            elif kind == "K" and g + 1 < NG:
                r = pl.ds(mult(t * 16 + (u // 2) * 8, 8), 8)
                nc = GC // 2
                c0 = (u % 2) * nc
                pltpu.make_async_copy(
                    wq_hbm.at[r, pl.ds((g + 1) * GC + c0, nc)],
                    wq_v.at[g + 1, r, pl.ds(c0, nc)], sem_h.at[2 * g]).start(priority=_HI)
                if g < 2:
                    stream(wo_hbm, wo_v, sem_e.at[0], WO0 + E_Q + g * E_K, S16, t, u)
            elif kind == "K":
                stream(wo_hbm, wo_v, sem_h.at[2 * g], WO0 + WO_E, S48, t, u)
            elif g + 1 < NG:
                src, dst = ffn[g]
                stream(src, dst, sem_h.at[2 * g + 1], 0, S40, t, u)
                stream(src, dst, sem_h.at[2 * g + 1], F1, (0, 0, 0, 8), t, u, t < F2T)
            else:
                stream(wo_hbm, wo_v, sem_h.at[2 * g + 1], WO0 + WO_E + WO_K, S32, t, u, t < V3T)
                stream(wo_hbm, wo_v, sem_o.at[0], -V3T * 32, S32, t, u,
                       between(t, V3T, V3T + NL))

        def step(kind, g, t, u):
            l_wait(kind, t, u)
            h_issue(kind, g, t, u)
            if kind == "Q":
                kv_start("K", 0, t, u)
            else:
                l_ahead(kind, g, t, u)

        def pick_rows(r):
            out = r[:, 0:DH]
            for i in range(1, G):
                out = jnp.where(row == i, r[:, i * DH:(i + 1) * DH], out)
            return out

        def qproj(g, k):
            r = jnp.dot(xn_s[k].astype(_BF16), wq_v[g, pl.ds(mult(k * 128, 128), 128), :],
                        preferred_element_type=_F32)
            return pick_rows(r)

        def xn_full():
            return jnp.concatenate([xn_s[k] for k in range(KD)], axis=1)

        def woproj(h):
            oh = jnp.broadcast_to(o_s[pl.ds(h, 1), :], (8, DH)).astype(_BF16)
            return jnp.dot(oh, wo_v[pl.ds(mult(h * DH, DH), DH), :],
                           preferred_element_type=_F32)

        x_cp = pltpu.make_async_copy(x_hbm, x_v, sem_x.at[0])
        wr_cp = pltpu.make_async_copy(wr_hbm, wr_v, sem_x.at[1])
        x_cp.start(priority=_HI)
        for t in range(KD):
            for u in range(SUB):
                q_start(t, u)
        wr_cp.start(priority=_HI)
        if FP > F:
            for _, dst in ffn:
                dst[pl.ds(F, FP - F), :] = jnp.zeros((FP - F, D), _BF16)
        y_s[...] = jnp.zeros((8, D), _F32)
        a_s[...] = jnp.zeros((8, D), _F32)

        x_cp.wait()
        x = x_v[0].astype(_F32)
        mu = jnp.mean(x, axis=-1, keepdims=True)
        xc = x - mu
        var = jnp.mean(xc * xc, axis=-1, keepdims=True)
        den = _rnd(jnp.sqrt(_rnd(_rnd(var) + 1e-5)))
        xn = _rnd(_rnd(x - _rnd(mu)) / den)
        xn8 = jnp.broadcast_to(xn, (8, D))
        for k in range(KD):
            xn_s[k] = xn8[:, k * 128:(k + 1) * 128]

        q = None
        for t in range(KD):
            for u in range(SUB):
                step("Q", 0, t, u)
            part = qproj(0, t)
            q = part if q is None else q + part
        q_s[...] = q

        for g in range(NG):
            def k_extra(t, g=g):
                if g == 0:
                    return
                w_v = ffn[g - 1][1]
                T0 = 2
                T1 = T0 + FT

                @pl.when(t == T0)
                def _():
                    wait_all(w_v.at[pl.ds(0, F), :], sem_h.at[2 * g - 1])

                @pl.when(between(t, T0, T1))
                def _():
                    idx = t - T0
                    w = w_v[pl.ds(pl.multiple_of(idx * 128, 128), 128), :]
                    if g == 1:
                        h_s[idx] = lax.dot_general(xn_full().astype(_BF16), w, _NT,
                                                   preferred_element_type=_F32)
                    elif g == 2:
                        up = lax.dot_general(xn_full().astype(_BF16), w, _NT,
                                             preferred_element_type=_F32)
                        gt = _rnd(h_s[idx])
                        h_s[idx] = _rnd(gt * jax.nn.sigmoid(gt)) * _rnd(up)
                    else:
                        y_s[...] += jnp.dot(h_s[idx].astype(_BF16), w,
                                            preferred_element_type=_F32)

                if g == 1:
                    @pl.when(between(t, T1, T1 + NO))
                    def _():
                        i = t - T1
                        oh = _rnd(o_s[pl.ds(i, 1), :])
                        ob_s[pl.ds(pl.multiple_of(i * DH, DH), DH), :] = jnp.transpose(
                            jnp.broadcast_to(oh, (DH, DH)))

                if g == NG - 1:
                    @pl.when(t == T1)
                    def _():
                        wr_cp.wait()
                        xf = xn_full()
                        r = jnp.sum(xf * wr_v[...].astype(_F32).reshape(1, D),
                                    axis=-1, keepdims=True)
                        r_sel = _rnd(jax.nn.sigmoid(_rnd(r)))
                        z = _rnd(xf + _rnd(_rnd(y_s[...]) * r_sel))
                        y_s[...] = _rnd(z * jax.nn.sigmoid(z))
                        wait_all(wo_v.at[pl.ds(WO0, WO_E), :], sem_e.at[0])

                    @pl.when(between(t, T1 + 1, T1 + 1 + HE - NO))
                    def _():
                        a_s[...] += woproj(t - (T1 + 1) + NO)

            qb = q_s[...].astype(_BF16)

            def k_body(t, m, g=g, qb=qb, k_extra=k_extra):
                step("K", g, t, 0)
                k_extra(t)
                for u in range(1, SUB):
                    step("K", g, t, u)
                kt = kbuf[:, pl.ds(pl.multiple_of(t * TR, TR), TR), :].reshape(G * TR, DH)
                s = pick_rows(lax.dot_general(qb, kt, _NT, preferred_element_type=_F32))
                s_s[t] = s
                return jnp.maximum(m, s)

            m_s[...] = lax.fori_loop(0, NT, k_body, jnp.full((G, DH), -jnp.inf, _F32))

            def v_extra(t, g=g):
                @pl.when(t == 0)
                def _():
                    m_s[...] = jnp.broadcast_to(
                        jnp.max(m_s[...], axis=-1, keepdims=True), (G, DH))

                @pl.when(t == 1)
                def _():
                    p = jnp.exp((s_s[...] - m_s[...][None]) * scale)
                    l = jnp.sum(jnp.sum(p, axis=0), axis=-1, keepdims=True)
                    il_s[...] = jnp.broadcast_to(1.0 / l, (G, DH))

                T0 = 2
                if g + 1 < NG:
                    @pl.when(t == T0)
                    def _():
                        wait_all(wq_v.at[g + 1], sem_h.at[2 * g])
                        q_s[...] = jnp.zeros((G, DH), _F32)

                    @pl.when(between(t, T0, T0 + KD))
                    def _():
                        q_s[...] += qproj(g + 1, t - T0)
                else:
                    @pl.when(t == T0)
                    def _():
                        wait_all(wo_v.at[pl.ds(WO0 + WO_E, WO_K), :], sem_h.at[2 * g])

                    @pl.when(between(t, T0, T0 + HL - HE))
                    def _():
                        a_s[...] += woproj(t - T0 + HE)

            def v_body(t, acc, g=g, v_extra=v_extra):
                step("V", g, t, 0)
                v_extra(t)
                for u in range(1, SUB):
                    step("V", g, t, u)
                r0 = pl.multiple_of(t * TR, TR)
                p = jnp.exp((s_s[t] - m_s[...]) * scale)
                vt = jnp.concatenate([vbuf[i, pl.ds(r0, TR), :] for i in range(G)], axis=1)
                r = jnp.dot(p.astype(_BF16), vt, preferred_element_type=_F32)
                return acc + pick_rows(r)

            acc = lax.fori_loop(0, NT, v_body, jnp.zeros((G, DH), _F32))
            o_s[pl.ds(g * G, G), :] = acc * il_s[...]

        wait_all(wo_v.at[pl.ds(WO0 + WO_E + WO_K, WO_V), :], sem_h.at[2 * NG - 1])
        part = None
        for reg in TREG:
            for s in reg:
                wait_all(wo_v.at[pl.ds(TOFF[s], TBLK[s]), :], sem_o.at[s])
            if part is None:
                a = a_s[...]
                for h in range(HL, H):
                    a = a + woproj(h)
                part = jnp.where(lax.broadcasted_iota(jnp.int32, (8, D), 0) == 0, a, 0.0)
            for s in reg:
                r = pl.ds(TOFF[s], TBLK[s])
                pr = wo_v[r, :].astype(_F32) * jnp.concatenate([ob_s[r, :]] * KD, axis=1)
                part = part + jnp.sum(pr.reshape(TBLK[s] // 8, 8, D), axis=0)
        att = jnp.sum(part, axis=0, keepdims=True)
        res = x_v[0].astype(_F32) + _rnd(_rnd(att) * y_s[0:1, :])
        o_ref[0] = res.astype(o_ref.dtype)

    scratch = [
        pltpu.VMEM((1, 1, D), _BF16),
        pltpu.VMEM((D,), _BF16),
        pltpu.VMEM((NG, D, GC), _BF16),
        pltpu.VMEM((H * DH, D), _BF16),
        pltpu.VMEM((FP, D), _BF16),
        pltpu.VMEM((FP, D), _BF16),
        pltpu.VMEM((FP, D), _BF16),
        pltpu.VMEM((G, W, DH), _BF16),
        pltpu.VMEM((G, W, DH), _BF16),
        pltpu.VMEM((KD, 8, 128), _F32),
        pltpu.VMEM((G, DH), _F32),
        pltpu.VMEM((NT, G, 128), _F32),
        pltpu.VMEM((G, DH), _F32),
        pltpu.VMEM((G, DH), _F32),
        pltpu.VMEM((H, DH), _F32),
        pltpu.VMEM((FT, 8, 128), _F32),
        pltpu.VMEM((8, D), _F32),
        pltpu.VMEM((8, D), _F32),
        pltpu.VMEM((NO * DH, DH), _F32),
        pltpu.SemaphoreType.DMA((DA * SUB,)),
        pltpu.SemaphoreType.DMA((2 * NG,)),
        pltpu.SemaphoreType.DMA((1,)),
        pltpu.SemaphoreType.DMA((len(TBLK),)),
        pltpu.SemaphoreType.DMA((2,)),
    ]
    return kernel, scratch


@jax.jit
def pallas_recurrent_scan__sliding_block_cached__moe_arch_mod__decode_kernel(
    A_x: jax.Array,
    A_k_cache: jax.Array,
    A_v_cache: jax.Array,
    A_wq: jax.Array,
    A_wo: jax.Array,
    B_x: jax.Array,
    B_w_r: jax.Array,
    B_w_gate: jax.Array,
    B_w_up: jax.Array,
    B_w_down: jax.Array,
):
    _, _, D = A_x.shape
    _, H, SK, DH = A_k_cache.shape
    W = min(4096, max(256, SK // 4))
    F = B_w_gate.shape[1]
    kernel, scratch = _make_kernel(D, H, SK, DH, W, F)
    hbm = pl.BlockSpec(memory_space=pltpu.MemorySpace.HBM)
    return pl.pallas_call(
        kernel,
        out_shape=jax.ShapeDtypeStruct(A_x.shape, A_x.dtype),
        in_specs=[hbm] * 9,
        out_specs=pl.BlockSpec(memory_space=pltpu.VMEM),
        scratch_shapes=scratch,
        compiler_params=pltpu.CompilerParams(
            vmem_limit_bytes=64 * 1024 * 1024,
            disable_bounds_checks=True,
            disable_semaphore_checks=True,
        ),
    )(A_x, A_k_cache, A_v_cache, A_wq, A_wo, B_w_r, B_w_gate.T, B_w_up.T, B_w_down)
```
